```python
import jax
import jax.numpy as jnp

def _softmax(x, axis=-1):
    return jax.nn.softmax(x, axis=axis)

def _gelu(x):
    return jax.nn.gelu(x, approximate=True)

def _silu(x):
    return jax.nn.silu(x)

def _sigmoid(x):
    return jax.nn.sigmoid(x)

def _layernorm(x, axis=-1, eps=1e-05):
    m = jnp.mean(x, axis=axis, keepdims=True)
    v = jnp.var(x, axis=axis, keepdims=True)
    return (x - m) / jnp.sqrt(v + eps)

def _scatter_add(tgt, idx, src, axis=0):
    return tgt.at[idx].add(src)

def _segment_sum(src, seg, n):
    return jax.ops.segment_sum(src, seg, n)

class _Rng:

    def __init__(self, key):
        self._k = key

    def _next(self):
        self._k, sub = jax.random.split(self._k)
        return sub

    def normal(self, shape):
        return jax.random.normal(self._next(), shape, dtype=jnp.bfloat16)

    def randint(self, lo, hi, shape):
        return jax.random.randint(self._next(), shape, lo, hi, dtype=jnp.int32)

    def uniform(self, shape, lo=0.0, hi=1.0):
        return jax.random.uniform(self._next(), shape, jnp.bfloat16, lo, hi)

    def permutation(self, n):
        return jax.random.permutation(self._next(), n)
kernel_name = 'concat_heads__ssm_conv_h3__memory_aug_infini_attn__prompt'

def setup_inputs():
    _rng = _Rng(jax.random.key(int.from_bytes(__import__("os").urandom(4), "little")))
    _w = lambda a: (lambda t: t.astype(jnp.bfloat16) if jnp.issubdtype(t.dtype, jnp.floating) else t)(jnp.asarray(a))

    def _A_setup():
        B, S, D = (1, 2048, 640)
        ks = 4
        return {'q': _w((lambda *s: _rng.normal(s) * 0.05)(B, S, D)), 'k': _w((lambda *s: _rng.normal(s) * 0.05)(B, S, D)), 'v': _w((lambda *s: _rng.normal(s) * 0.05)(B, S, D)), 'shift_k': _w((lambda *s: _rng.normal(s) * 0.05)(D, ks) * 0.5), 'ssm_k': _w((lambda *s: _rng.normal(s) * 0.05)(D, S) * (1.0 / S ** 0.5)), 'ssm_D': _w((lambda *s: _rng.normal(s) * 0.05)(D))}
    _A_in = _A_setup()

    def _B_setup():
        B, S, D, H = (1, 2048, 640, 32)
        N = 4
        L = max(1, S // N)
        sc = D ** (-0.5)
        return {'x': _w((lambda *s: _rng.normal(s) * 0.05)(B, N * L, D)), 'wq': _w((lambda *s: _rng.normal(s) * 0.05)(D, D) * sc), 'wk': _w((lambda *s: _rng.normal(s) * 0.05)(D, D) * sc), 'wv': _w((lambda *s: _rng.normal(s) * 0.05)(D, D) * sc), 'wo': _w((lambda *s: _rng.normal(s) * 0.05)(D, D) * sc), 'beta': _w((lambda *s: _rng.normal(s) * 0.05)(H))}
    _B_in = _B_setup()
    return {'A_q': _A_in['q'], 'A_k': _A_in['k'], 'A_v': _A_in['v'], 'A_shift_k': _A_in['shift_k'], 'A_ssm_k': _A_in['ssm_k'], 'A_ssm_D': _A_in['ssm_D'], 'B_x': _B_in['x'], 'B_wq': _B_in['wq'], 'B_wk': _B_in['wk'], 'B_wv': _B_in['wv'], 'B_wo': _B_in['wo'], 'B_beta': _B_in['beta']}

def reference(A_q, A_k, A_v, A_shift_k, A_ssm_k, A_ssm_D, B_x, B_wq, B_wk, B_wv, B_wo, B_beta):

    def _A_ref(q, k, v, shift_k, ssm_k, ssm_D):
        B, S, D = q.shape
        ks = shift_k.shape[-1]
        k_pad = jnp.pad(k, ((0, 0), (ks - 1, 0), (0, 0)))
        k_shift = jnp.zeros_like(k)
        for t in range(ks):
            k_shift = k_shift + k_pad[:, t:t + S, :] * shift_k[:, ks - 1 - t][None, None, :]
        kv = k_shift * v
        L = 2 * S
        kv_pad = jnp.pad(kv, ((0, 0), (0, S), (0, 0)))
        kf_pad = jnp.pad(ssm_k, ((0, 0), (0, S)))
        kv_f = (lambda x, axes=(-2, -1): jnp.fft.rfft2(x.astype(jnp.float32), axes=axes))(kv_pad[:, None, :, :], axes=(1, 2))
        kf_f = (lambda x, axes=(-2, -1): jnp.fft.rfft2(x.astype(jnp.float32), axes=axes))(kf_pad[:, None, :], axes=(1, 2))
        kf_f = (lambda x, *d: x.transpose(*d))(kf_f, 1, 2, 0)
        y_f = kv_f * kf_f[None, :, :, :]
        y = (lambda x, s, axes=(-2, -1): jnp.fft.irfft2(x, s=s, axes=axes).astype(jnp.bfloat16))(y_f, (1, L), axes=(1, 2))[:, 0, :S, :]
        y = y + kv * ssm_D[None, None, :]
        return q * y

    def _B_ref(x, wq, wk, wv, wo, beta):
        B, S, D = x.shape
        H = 32
        Dh = D // H
        N = 4
        L = S // N
        q = (lambda x, *d: x.transpose(*d))((x @ wq).reshape(B, S, H, Dh), 0, 2, 1, 3).reshape(B, H, N, L, Dh)
        k = (lambda x, *d: x.transpose(*d))((x @ wk).reshape(B, S, H, Dh), 0, 2, 1, 3).reshape(B, H, N, L, Dh)
        v = (lambda x, *d: x.transpose(*d))((x @ wv).reshape(B, S, H, Dh), 0, 2, 1, 3).reshape(B, H, N, L, Dh)
        phi = lambda t: jnp.where(t > 0, t + 1.0, jnp.exp(t))
        scale = Dh ** (-0.5)
        ar = jnp.arange(L)
        mask = (lambda x, dt: x.astype(dt))(ar[:, None] < ar[None, :], x.dtype) * -1000000000.0
        g = _sigmoid(beta).reshape(1, H, 1, 1)
        M = jnp.einsum('bhd,bhe->bhde', q[:, :, 0, 0, :] * 0.0, q[:, :, 0, 0, :] * 0.0)
        z = q[:, :, 0, 0, :] * 0.0
        outs = []
        for s in range(N):
            qs, ks, vs = (q[:, :, s].copy(), k[:, :, s].copy(), v[:, :, s].copy())
            logits = jnp.einsum('bhqd,bhkd->bhqk', qs, ks) * scale + mask
            p = _softmax(logits, axis=-1)
            a_dot = jnp.einsum('bhqk,bhkd->bhqd', p, vs)
            pq = phi(qs)
            num = jnp.einsum('bhld,bhde->bhle', pq, M)
            den = jnp.einsum('bhld,bhd->bhl', pq, z)[..., None] + 1e-06
            a_mem = num / den
            o = g * a_mem + (1.0 - g) * a_dot
            outs.append(o)
            pk = phi(ks)
            M = M + jnp.einsum('bhld,bhle->bhde', pk, vs)
            z = z + jnp.einsum('bhld->bhd', pk)
        o = (lambda x, *d: x.transpose(*d))(jnp.stack(outs, 2).reshape(B, H, S, Dh), 0, 2, 1, 3).reshape(B, S, D)
        return o @ wo
    a = _A_ref(A_q, A_k, A_v, A_shift_k, A_ssm_k, A_ssm_D)
    b = _B_ref(B_x, B_wq, B_wk, B_wv, B_wo, B_beta)
    return jnp.concatenate([a, b], axis=-1)
```

```python
import functools
import math

import jax
import jax.numpy as jnp
import numpy as np
from jax import lax
import jax.experimental.pallas as pl
import jax.experimental.pallas.tpu as pltpu

BF = jnp.bfloat16
F32 = jnp.float32
U32 = jnp.uint32
I32 = jnp.int32

S = 2048
D = 640
H = 32
DH = 20
NSEG = 4
L = S // NSEG
T = 128
NB = S // T
NG = D // T
LOG2E = 1.4426950408889634
QSCALE = DH ** -0.5 * LOG2E
NEG = -1e9 * LOG2E

CFG = dict(nh=8, lagB=12, lagC=8, G=4)


def _dft_matrices():
    m = np.arange(T)
    theta = (0.5 * np.pi + 2.0 * np.pi * m) / T
    ang = theta[:, None] * np.arange(T)[None, :]
    f = np.stack([np.cos(ang).reshape(NB, 8, T), np.sin(ang).reshape(NB, 8, T)], axis=1)
    f = f.reshape(2 * T, T)
    return f.astype(BF), (f.T / T).astype(BF)


_FWD, _INV = _dft_matrices()

_H0 = [(T * w) // DH for w in range(NG)]
_H1 = [(T * w + T - 1) // DH for w in range(NG)]
_R0 = [(DH * h) // 8 * 8 for h in _H0]
_R1 = [-(-(DH * (h + 1)) // 8) * 8 for h in _H1]


def _phi(t):
    return jnp.where(t > 0, t + 1.0, jnp.exp(t))


def _head_of(idx):
    return (idx * 3277) >> 16


def _short_conv(us, ks):
    out = []
    for c in range(NB):
        acc = us[c] * ks[0]
        for j in range(1, c + 1):
            acc = acc + us[c - j] * ks[j]
        out.append(acc)
    return out


def _kernel(aq_hbm, ak_hbm, av_hbm, sk_ref, fk_hbm, dd_ref, x_hbm, wq_hbm, wk_hbm, wv_hbm,
            wo_hbm, beta_ref, fwd_ref, inv_ref, out_hbm,
            aq_v, ak_v, av_v, fk_v, x_v, wq_v, wk_v, wv_v, wo_v,
            kv_s, uf_s, kf_s, z_s, ya_s,
            k_s, q_s, v_s, pk_s, pq_s, num_s, rden_s, ot_s, yb_s, mask_s, par_s, g_s,
            sem_in, sem_a, sem_out):
    cfg = CFG

    def cp_x():
        return pltpu.make_async_copy(x_hbm, x_v, sem_in.at[0])

    def cp_w(i):
        src, dst = ((wq_hbm, wq_v), (wk_hbm, wk_v), (wv_hbm, wv_v))[i]
        return [pltpu.make_async_copy(src.at[:, T * g:T * (g + 1)], dst.at[g], sem_in.at[1 + i])
                for g in range(NG)]

    def cp_wo():
        return pltpu.make_async_copy(wo_hbm, wo_v, sem_in.at[4])

    def cp_a(i, g):
        c0 = pl.multiple_of(g * T, T)
        if i == 3:
            return pltpu.make_async_copy(fk_hbm.at[pl.ds(c0, T), :], fk_v.at[g], sem_a.at[3, g])
        src, dst = ((ak_hbm, ak_v), (av_hbm, av_v), (aq_hbm, aq_v))[i]
        return pltpu.make_async_copy(src.at[:, pl.ds(c0, T)], dst.at[g], sem_a.at[i, g])

    def cp_ya(g):
        c0 = pl.multiple_of(g * T, T)
        return pltpu.make_async_copy(ya_s.at[g], out_hbm.at[:, pl.ds(c0, T)], sem_out.at[g])

    def cp_yb(s):
        r0 = pl.multiple_of(s * L, L)
        return pltpu.make_async_copy(yb_s.at[s], out_hbm.at[pl.ds(r0, L), D:2 * D], sem_out.at[NG + s])

    cp_a(3, 0).start()
    cp_a(0, 0).start()
    cp_a(1, 0).start()
    cp_x().start()
    for i in range(3):
        for c in cp_w(i):
            c.start()
    cp_a(2, 0).start()
    for g in range(1, NG):
        for i in (3, 0, 1, 2):
            cp_a(i, g).start()
    cp_wo().start()

    r_i = lax.broadcasted_iota(I32, (T, T), 0)
    c_i = lax.broadcasted_iota(I32, (T, T), 1)
    mask_s[...] = jnp.where(r_i <= c_i, 0.0, NEG)
    taps = sk_ref[...].astype(F32)
    dvec = dd_ref[...].astype(F32).reshape(1, D)
    for g in range(NG):
        for j in range(4):
            par_s[g, j] = jnp.broadcast_to(taps[j:j + 1, T * g:T * (g + 1)], (8, T))
        par_s[g, 4] = jnp.broadcast_to(dvec[:, T * g:T * (g + 1)], (8, T))
    gate = jax.nn.sigmoid(beta_ref[...].astype(F32).reshape(1, H)).astype(BF).astype(F32)
    hr = lax.broadcasted_iota(I32, (H, H), 0)
    hc = lax.broadcasted_iota(I32, (H, H), 1)
    gcol = jnp.sum(jnp.where(hr == hc, jnp.broadcast_to(gate, (H, H)), 0.0), axis=1, keepdims=True)
    g_s[...] = jnp.broadcast_to(gcol, (H, T))

    cp_x().wait()
    for i in range(3):
        for c in cp_w(i):
            c.wait()

    def phase1(g, carry):
        for i in (3, 0, 1, 2):
            cp_a(i, g).wait()
        fwd = fwd_ref[...]

        def filt(j):
            kf_s[j] = lax.dot_general(fwd, fk_v[g, :, T * j:T * (j + 1)], (((1,), (1,)), ((), ())),
                                      preferred_element_type=F32)

        def kv(a):
            cur = ak_v[g, T * a:T * (a + 1), :].astype(F32)
            if a == 0:
                prev = jnp.zeros((8, T), F32)
            else:
                prev = ak_v[g, T * a - 16:T * a, :].astype(F32)[8:]
            ext = jnp.concatenate([prev, cur], axis=0)
            acc = cur * par_s[g, 0][0:1]
            for j in range(1, 4):
                acc = acc + ext[8 - j:8 - j + T] * par_s[g, j][0:1]
            u = (acc * av_v[g, T * a:T * (a + 1), :].astype(F32)).astype(BF)
            kv_s[T * a:T * (a + 1), :] = u
            uf_s[a] = jnp.dot(fwd, u, preferred_element_type=F32)

        def slab(s):
            re, im = slice(16 * s, 16 * s + 8), slice(16 * s + 8, 16 * s + 16)
            kr = [kf_s[j, re, :] for j in range(NB)]
            ki = [kf_s[j, im, :] for j in range(NB)]
            fr = [kr[0]] + [kr[j] + ki[j - 1] for j in range(1, NB)]
            fi = [ki[0]] + [ki[j] - kr[j - 1] for j in range(1, NB)]
            ur = [uf_s[a, re, :] for a in range(NB)]
            ui = [uf_s[a, im, :] for a in range(NB)]
            t1 = _short_conv([ur[a] + ui[a] for a in range(NB)], fr)
            t2 = _short_conv(ur, [fi[j] - fr[j] for j in range(NB)])
            t3 = _short_conv(ui, [fr[j] + fi[j] for j in range(NB)])
            for c in range(NB):
                zz = jnp.concatenate([t1[c] - t3[c], t1[c] + t2[c]], axis=0)
                z_s[c, 16 * s:16 * s + 16, :] = zz.astype(BF)

        def inv(c):
            y = jnp.dot(inv_ref[...], z_s[c], preferred_element_type=F32)
            rows = slice(T * c, T * (c + 1))
            y = y + kv_s[rows, :].astype(F32) * par_s[g, 4][0:1]
            ya_s[g, rows, :] = (aq_v[g, rows, :].astype(F32) * y).astype(BF)

        wqv_t = jnp.concatenate([wq_v[g].T, wv_v[g].T], axis=0)
        gp = jnp.maximum(g - 1, 0)

        def proj_k(t):
            rows = slice(T * t, T * (t + 1))
            k = jnp.dot(x_v[rows, :], wk_v[g], preferred_element_type=F32)
            kb = k.astype(BF)
            k_s[g, rows, :] = kb
            pk_s[g, rows, :] = _phi(k).astype(BF)
            k_s[NG + g, rows, :] = jnp.where(c_i < 64, kb, k_s[gp, rows, :])

        def proj_qv(t):
            cols = slice(T * t, T * (t + 1))
            qv = lax.dot_general(wqv_t, x_v[cols, :], (((1,), (1,)), ((), ())),
                                 preferred_element_type=F32)
            r0 = pl.multiple_of(g * T, T)
            q = qv[:T]
            q_s[pl.ds(r0, T), cols] = (q * QSCALE).astype(BF)
            pq_s[g, :, cols] = _phi(q).astype(BF)
            v_s[pl.ds(r0, T), cols] = qv[T:]

        for j in range(NB):
            filt(j)
            kv(j)
        for s in range(NB):
            proj_k(s)
            proj_qv(s)
            slab(s)
        for c in range(NB):
            inv(c)
        cp_ya(g).start()
        return carry

    lax.fori_loop(0, NG, phase1, 0)

    gcolv = g_s[...]
    num_s[0] = jnp.zeros((D, L), F32)
    for i in range(L // T):
        rden_s[i] = jnp.zeros((H, T), F32)
    mem = [None] * NG
    for s in range(NSEG - 1):
        tok = slice(L * s, L * (s + 1))
        lhs = []
        for w in range(NG):
            n = _R1[w] - _R0[w]
            vv = jnp.concatenate([v_s[_R0[w]:_R1[w], tok], jnp.ones((8, L), F32)], axis=0)
            upd = lax.dot_general(vv, pk_s[w, tok, :], (((1,), (0,)), ((), ())),
                                  preferred_element_type=F32)
            mem[w] = upd if mem[w] is None else mem[w] + upd
            rh = _head_of(lax.broadcasted_iota(I32, (n, T), 0) + _R0[w])
            ch = _head_of(lax.broadcasted_iota(I32, (n, T), 1) + T * w)
            zh = lax.broadcasted_iota(I32, (8, T), 0) + _H0[w]
            ch8 = _head_of(lax.broadcasted_iota(I32, (8, T), 1) + T * w)
            lhs.append(jnp.concatenate([jnp.where(rh == ch, mem[w][:n], 0.0),
                                        jnp.where(zh == ch8, mem[w][n:], 0.0)], axis=0))
        tok = slice(L * (s + 1), L * (s + 2))
        res = [lax.dot_general(lhs[w], pq_s[w, :, tok], (((1,), (0,)), ((), ())),
                               preferred_element_type=F32) for w in range(NG)]
        for w in range(NG):
            lo = _R0[w] if w == 0 else _R1[w - 1]
            hi = _R1[w] if w == NG - 1 else _R0[w + 1]
            num_s[s + 1, lo:hi, :] = res[w][lo - _R0[w]:hi - _R0[w]]
            if w + 1 < NG:
                num_s[s + 1, hi:_R1[w], :] = (res[w][hi - _R0[w]:_R1[w] - _R0[w]]
                                              + res[w + 1][:_R1[w] - hi])
        dens = [res[w][_R1[w] - _R0[w]:] for w in range(NG)]
        pad = [jnp.concatenate(
            ([jnp.zeros((_H0[w], L), F32)] if _H0[w] else []) + [dens[w]]
            + [jnp.zeros((40 - 8 - _H0[w], L), F32)], axis=0) for w in range(NG)]
        den = (pad[0] + pad[1] + pad[2] + pad[3] + pad[4])[:H]
        for i in range(L // T):
            rden_s[(s + 1) * (L // T) + i] = gcolv / (den[:, T * i:T * (i + 1)] + 1e-6)

    cp_wo().wait()

    nh = cfg["nh"]
    tiles = [(r, i, j) for r in range(nh) for i in range(L // T) for j in range(i + 1)]
    row_t = lax.broadcasted_iota(I32, (T, T), 0)
    sub8 = lax.broadcasted_iota(I32, (8, T), 0)

    def heads(s, m):
        t0 = pl.multiple_of(s * L, L)
        qws, mx, svals, pvals, acc, fin, held = {}, {}, {}, {}, {}, {}, {}

        def stage_a(t):
            r, i, j = tiles[t]
            h = m * nh + r
            f0 = h * DH
            wb = f0 >> 7
            wa = (f0 + DH - 1) >> 7
            kwin = jnp.where(wa == wb, wb, NG + wa)
            if (r, i) not in qws:
                cols = pl.ds(pl.multiple_of(t0 + T * i, T), T)
                qq = jnp.concatenate([
                    q_s[pl.ds(pl.multiple_of(wa * T, T), 64), cols],
                    q_s[pl.ds(pl.multiple_of(wb * T + 64, 64), 64), cols]], axis=0)
                qws[(r, i)] = jnp.where(((row_t - f0) & (T - 1)) < DH, qq, jnp.zeros_like(qq))
            kw = k_s[kwin, pl.ds(pl.multiple_of(t0 + T * j, T), T), :]
            sc = jnp.dot(kw, qws[(r, i)], preferred_element_type=F32)
            if i == j:
                sc = sc + mask_s[...]
            m8 = jnp.max(sc.reshape(16, 8, T), axis=0)
            mx[(r, i)] = m8 if (r, i) not in mx else jnp.maximum(mx[(r, i)], m8)
            svals[t] = sc

        def stage_b(t):
            r, i, j = tiles[t]
            if (r, i) not in fin:
                fin[(r, i)] = jnp.max(mx[(r, i)], axis=0, keepdims=True)
            pvals[t] = jnp.exp2(svals.pop(t) - fin[(r, i)]).astype(BF)

        def stage_c(t):
            r, i, j = tiles[t]
            h = m * nh + r
            pair = pl.multiple_of((m * (nh // 2) + r // 2) * 40, 8)
            base = pl.multiple_of(pair + (r % 2) * 16, 8)
            vv = v_s[pl.ds(base, 24), pl.ds(pl.multiple_of(t0 + T * j, T), T)]
            if r % 2 == 0:
                vv = jnp.concatenate([vv[:16], jnp.where(sub8 < 4, vv[16:], 1.0)], axis=0)
            else:
                vv = jnp.concatenate([jnp.where(sub8 >= 4, vv[:8], 1.0), vv[8:]], axis=0)
            o = lax.dot_general(vv, pvals.pop(t), (((1,), (0,)), ((), ())),
                                preferred_element_type=F32)
            acc[(r, i)] = o if (r, i) not in acc else acc[(r, i)] + o
            if i == j:
                a = acc.pop((r, i))
                cols = slice(T * i, T * (i + 1))
                den = a[20:21] if r % 2 == 0 else a[0:1]
                w_dot = (1.0 - g_s[pl.ds(h, 1), :]) / den
                w_mem = rden_s[s * (L // T) + i, pl.ds(h, 1), :]
                o = a * w_dot + num_s[s, pl.ds(base, 24), cols] * w_mem
                if r % 2 == 0:
                    ot_s[pl.ds(base, 16), cols] = o[:16]
                    held[(r, i)] = o[16:]
                else:
                    mid = jnp.where(sub8 < 4, held.pop((r - 1, i)), o[:8])
                    ot_s[pl.ds(base, 24), cols] = jnp.concatenate([mid, o[8:]], axis=0)

        n = len(tiles)
        lb, lc, grp = cfg["lagB"], cfg["lagC"], cfg["G"]
        for tt in range(0, n + lb + lc, grp):
            for t in range(tt, tt + grp):
                if t < n:
                    stage_a(t)
            for t in range(tt, tt + grp):
                if 0 <= t - lb < n:
                    stage_b(t - lb)
            for t in range(tt, tt + grp):
                if 0 <= t - lb - lc < n:
                    stage_c(t - lb - lc)

    def segment(s, carry):
        def body(m, c):
            heads(s, m)
            return c
        lax.fori_loop(0, H // nh, body, 0)
        ot = ot_s[...].astype(BF)
        yb_s[s] = lax.dot_general(ot, wo_v[...], (((0,), (0,)), ((), ())),
                                  preferred_element_type=F32).astype(BF)
        cp_yb(s).start()
        return carry

    lax.fori_loop(0, NSEG, segment, 0)

    for g in range(NG):
        cp_ya(g).wait()
    for s in range(NSEG):
        cp_yb(s).wait()


@jax.jit
def pallas_concat_heads__ssm_conv_h3__memory_aug_infini_attn__prompt_kernel(
    A_q, A_k, A_v, A_shift_k, A_ssm_k, A_ssm_D, B_x, B_wq, B_wk, B_wv, B_wo, B_beta,
):
    hbm = pl.BlockSpec(memory_space=pl.ANY)
    vmem = pl.BlockSpec(memory_space=pltpu.VMEM)
    scratch = [
        pltpu.VMEM((NG, S, T), BF),
        pltpu.VMEM((NG, S, T), BF),
        pltpu.VMEM((NG, S, T), BF),
        pltpu.VMEM((NG, T, S), BF),
        pltpu.VMEM((S, D), BF),
        pltpu.VMEM((NG, D, T), BF),
        pltpu.VMEM((NG, D, T), BF),
        pltpu.VMEM((NG, D, T), BF),
        pltpu.VMEM((D, D), BF),
        pltpu.VMEM((S, T), BF),
        pltpu.VMEM((NB, 2 * T, T), F32),
        pltpu.VMEM((NB, 2 * T, T), F32),
        pltpu.VMEM((NB, 2 * T, T), BF),
        pltpu.VMEM((NG, S, T), BF),
        pltpu.VMEM((2 * NG, S, T), BF),
        pltpu.VMEM((D, S), BF),
        pltpu.VMEM((D, S), F32),
        pltpu.VMEM((NG, S, T), BF),
        pltpu.VMEM((NG, T, S), BF),
        pltpu.VMEM((NSEG, D, L), F32),
        pltpu.VMEM((S // T, H, T), F32),
        pltpu.VMEM((D, L), F32),
        pltpu.VMEM((NSEG, L, D), BF),
        pltpu.VMEM((T, T), F32),
        pltpu.VMEM((NG, 5, 8, T), F32),
        pltpu.VMEM((H, T), F32),
        pltpu.SemaphoreType.DMA((5,)),
        pltpu.SemaphoreType.DMA((4, NG)),
        pltpu.SemaphoreType.DMA((NG + NSEG,)),
    ]
    out = pl.pallas_call(
        _kernel,
        out_shape=jax.ShapeDtypeStruct((S, 2 * D), BF),
        in_specs=[hbm, hbm, hbm, vmem, hbm, vmem, hbm, hbm, hbm, hbm, hbm, vmem, vmem, vmem],
        out_specs=hbm,
        scratch_shapes=scratch,
        compiler_params=pltpu.CompilerParams(vmem_limit_bytes=100 * 1024 * 1024),
        name="h3_infini",
    )(A_q.reshape(S, D), A_k.reshape(S, D), A_v.reshape(S, D), A_shift_k.T, A_ssm_k, A_ssm_D,
      B_x.reshape(S, D), B_wq, B_wk, B_wv, B_wo, B_beta, _FWD, _INV)
    return out.reshape(1, S, 2 * D)
```

```python
import jax
import jax.numpy as jnp
import numpy as np
from jax import lax
import jax.experimental.pallas as pl
import jax.experimental.pallas.tpu as pltpu

BF = jnp.bfloat16
F32 = jnp.float32
U32 = jnp.uint32
I32 = jnp.int32

S = 2048
D = 640
H = 32
DH = 20
NSEG = 4
L = S // NSEG
T = 128
NB = S // T
NQ = L // T
NG = D // T
RING = 24
LOG2E = 1.4426950408889634
QSCALE = DH ** -0.5 * LOG2E
NEG = -1e9 * LOG2E

CFG = dict(tr=4, parts='', fu=1, xw=2, wt0=1, p2=1, lagB=8, lagC=4, G=2, iorder=(0, 1, 2, 3), olag=8, inv_at=16, slabs=[1] * 16, scopes=False)


def _dft_matrices():
    theta = (0.5 * np.pi + 2.0 * np.pi * np.arange(T)) / T
    ang = theta[:, None] * np.arange(T)[None, :]
    f = np.stack([np.cos(ang).reshape(NB, 8, T), np.sin(ang).reshape(NB, 8, T)], axis=1)
    f = f.reshape(2 * T, T)
    g = (f.T / T).reshape(T, 2, T).transpose(1, 0, 2).reshape(2 * T, T)
    return np.concatenate([f, g], axis=0).astype(BF)


_DFT = _dft_matrices()

_H0 = [(T * w) // DH for w in range(NG)]
_H1 = [(T * w + T - 1) // DH for w in range(NG)]
_R0 = [(DH * h) // 8 * 8 for h in _H0]
_R1 = [-(-(DH * (h + 1)) // 8) * 8 for h in _H1]


def _phi(t):
    return jnp.where(t > 0, t + 1.0, jnp.exp(t))


def _head_of(idx):
    return (idx * 3277) >> 16


def _ld(ref, idx, r0, n):
    if isinstance(r0, int):
        rows = pl.ds(r0 // 2, n // 2)
    else:
        rows = pl.ds(pl.multiple_of(r0 // 2, 8), n // 2)
    return pltpu.bitcast(ref.bitcast(U32)[(*idx, rows, slice(None))], BF)


def _nn(a, b):
    return lax.dot_general(a, b, (((1,), (0,)), ((), ())), preferred_element_type=F32)


def _nt(a, b):
    return lax.dot_general(a, b, (((1,), (1,)), ((), ())), preferred_element_type=F32)


def _short_conv(us, ks):
    out = []
    for c in range(NB):
        acc = us[c] * ks[0]
        for j in range(1, c + 1):
            acc = acc + us[c - j] * ks[j]
        out.append(acc)
    return out


def _start(copies):
    for c in copies:
        c.start()


def _wait(copies):
    for c in copies:
        c.wait()


def _scope(name):
    return jax.named_scope(name) if CFG["scopes"] else _NoScope()


class _NoScope:
    def __enter__(self):
        return None

    def __exit__(self, *exc):
        return False


def _kernel(aq_hbm, ak_hbm, av_hbm, sk_hbm, fk_hbm, dd_hbm, x_hbm, wq_hbm, wk_hbm, wv_hbm,
            wo_hbm, beta_hbm, dft_hbm, out_hbm,
            aq_v, ak_v, av_v, fk_v, x_v, wq_v, wk_v, wv_v, wo_v, sk_v, dd_v, beta_v, dft_v,
            wt_s, kv_s, uf_s, kf_s, z_s, ya_s,
            k_s, q_s, v_s, pk_s, pq_s, num_s, rden_s, yb_s, mask_s, par_s, g_s, zero_s,
            sem_s, sem_g, sem_out, *rest):
    cfg = CFG
    ot_s, s_ring, t_ring = rest[:NQ], rest[NQ:NQ + RING], rest[NQ + RING:]

    def col(g):
        return pl.ds(g * T if isinstance(g, int) else pl.multiple_of(g * T, T), T)

    def cp_small():
        return [pltpu.make_async_copy(src, dst, sem_s.at[0]) for src, dst in
                ((sk_hbm, sk_v), (dd_hbm, dd_v), (beta_hbm, beta_v), (dft_hbm, dft_v))]

    def cp_x(c):
        rows = pl.ds(c * L, L)
        return [pltpu.make_async_copy(x_hbm.at[rows, col(w)], x_v.at[w, rows], sem_s.at[1 + c])
                for w in range(NG)]

    def cp_wo():
        return [pltpu.make_async_copy(wo_hbm.at[:, col(w)], wo_v.at[w], sem_s.at[1 + NSEG])
                for w in range(NG)]

    def src_group(g):
        return min(g, NG - 1) if isinstance(g, int) else jnp.minimum(g, NG - 1)

    def cp_f(g):
        return [pltpu.make_async_copy(fk_hbm.at[col(src_group(g)), :], fk_v.at[g], sem_g.at[g])]

    def cp_u(g):
        return [pltpu.make_async_copy(src.at[:, col(src_group(g))], dst.at[g], sem_g.at[NG + 1 + g])
                for src, dst in ((ak_hbm, ak_v), (av_hbm, av_v))]

    def cp_q(g):
        return [pltpu.make_async_copy(aq_hbm.at[:, col(src_group(g))], aq_v.at[g], sem_g.at[2 * NG + 2 + g])]

    def cp_conv(g):
        return cp_f(g) + cp_u(g) + cp_q(g)

    def cp_w(g):
        return [pltpu.make_async_copy(src.at[:, col(g)], dst.at[g], sem_g.at[3 * NG + 3 + g])
                for src, dst in ((wq_hbm, wq_v), (wk_hbm, wk_v), (wv_hbm, wv_v))]

    def cp_ya(g):
        return pltpu.make_async_copy(ya_s.at[g], out_hbm.at[:, col(g)], sem_out.at[g])

    def cp_yb(s):
        r0 = s * L if isinstance(s, int) else pl.multiple_of(s * L, L)
        return pltpu.make_async_copy(yb_s.at[s], out_hbm.at[pl.ds(r0, L), D:2 * D], sem_out.at[NG + s])

    _start(cp_x(0) + cp_w(0) + cp_small())

    for i in range(8):
        zero_s[i] = 0
    r_i = lax.broadcasted_iota(I32, (T, T), 0)
    c_i = lax.broadcasted_iota(I32, (T, T), 1)
    mask_s[...] = jnp.where(r_i <= c_i, 0.0, NEG)

    def x_tile(t):
        return jnp.concatenate([_ld(x_v, (c,), T * t, T) for c in range(NG)], axis=1)

    def transpose_w(g):
        for c in range(NG):
            wt_s[g, c, 0:T, :] = _ld(wq_v, (g,), T * c, T).T
            wt_s[g, c, T:2 * T, :] = _ld(wv_v, (g,), T * c, T).T

    def proj(g, t, z):
        rows = slice(T * t, T * (t + 1))
        words = slice(T * t // 2, T * (t + 1) // 2)
        k = _nn(x_tile(t), _ld(wk_v, (g,), 0, D))
        k_s[g, rows, :] = k.astype(BF)
        pk_s[g, rows, :] = _phi(k).astype(BF)
        if not isinstance(g, int) or g:
            gp = g - 1 if isinstance(g, int) else jnp.maximum(g - 1, 0)
            ku = k_s.bitcast(U32)
            ku[NG + g, words, :] = jnp.where(c_i[:T // 2] < 64, ku[g + z, words, :], ku[gp + z, words, :])
        wt = jnp.concatenate([_ld(wt_s, (g + z, c), 0, 2 * T) for c in range(NG)], axis=1)
        qv = _nt(wt, x_tile(t))
        q = qv[:T]
        q_s[t, col(g), :] = (q * QSCALE).astype(BF)
        pq_s[t, col(g), :] = _phi(q).astype(BF)
        v_s[t, col(g), :] = qv[T:]

    with _scope("ph_wait0"):
        _wait(cp_x(0) + cp_w(0))
    with _scope("ph_10"):
        z0 = zero_s[0]
        for g in range(NG):
            if g == 0:
                _start(cp_w(1))
                transpose_w(0)
            elif g == 1:
                _start(cp_w(2) + cp_w(3) + cp_w(4))
                _wait(cp_w(1))
                transpose_w(1)
            elif g == 2:
                _start(cp_x(1) + cp_x(2) + cp_x(3) + cp_conv(0))
                _wait(cp_w(2) + cp_w(3) + cp_w(4))
                transpose_w(2)
            if 2 <= g < NG - 1:
                transpose_w(g + 1)
            for t in range(NQ):
                proj(g, t, z0)

        _wait(cp_small())
        taps = sk_v[...].astype(F32)
        dvec = dd_v[...].astype(F32).reshape(1, D)
        for g in range(NG):
            for j in range(4):
                par_s[g, j] = jnp.broadcast_to(taps[j:j + 1, T * g:T * (g + 1)], (8, T))
            par_s[g, 4] = jnp.broadcast_to(dvec[:, T * g:T * (g + 1)], (8, T))
        gate = jax.nn.sigmoid(beta_v[...].astype(F32).reshape(1, H)).astype(BF).astype(F32)
        hr = lax.broadcasted_iota(I32, (H, H), 0)
        hc = lax.broadcasted_iota(I32, (H, H), 1)
        gcol = jnp.sum(jnp.where(hr == hc, jnp.broadcast_to(gate, (H, H)), 0.0), axis=1, keepdims=True)
        g_s[...] = jnp.broadcast_to(gcol, (H, T))
        _wait(cp_x(1) + cp_x(2) + cp_x(3))

    def phase1(g, carry):
        _start(cp_conv(g + 1))
        with _scope('ph_wg'):
            _wait(cp_conv(g))
        zeros = [zero_s[i] for i in range(5)]
        fwd = lambda: _ld(dft_v, (), 0, 2 * T)

        def filt(j):
            kf_s[j] = _nt(fwd(), fk_v[g, :, T * j:T * (j + 1)])

        def kv(a):
            cur = _ld(ak_v, (g,), T * a, T).astype(F32)
            if a == 0:
                prev = jnp.zeros((8, T), F32)
            else:
                prev = _ld(ak_v, (g,), T * a - 16, 16).astype(F32)[8:]
            ext = jnp.concatenate([prev, cur], axis=0)
            acc = cur * par_s[g, 0][0:1]
            for j in range(1, 4):
                acc = acc + ext[8 - j:8 - j + T] * par_s[g, j][0:1]
            u = (acc * _ld(av_v, (g,), T * a, T).astype(F32)).astype(BF)
            kv_s[T * a:T * (a + 1), :] = u
            uf_s[a] = _nn(fwd(), u)

        def slab(s):
            re, im = slice(16 * s, 16 * s + 8), slice(16 * s + 8, 16 * s + 16)
            t1_s, t2_s = t_ring[2 * (s % cfg['tr'])], t_ring[2 * (s % cfg['tr']) + 1]
            for part, dst, z in ((re, t1_s, zeros[0]), (im, t2_s, zeros[1])):
                t = _short_conv([uf_s[a + z, part, :] for a in range(NB)],
                                [kf_s[j + z, part, :] for j in range(NB)])
                for c in range(NB):
                    dst[0, c] = t[c]
            z = zeros[2]
            t = _short_conv([uf_s[a + z, re, :] + uf_s[a + z, im, :] for a in range(NB)],
                            [kf_s[j + z, re, :] + kf_s[j + z, im, :] for j in range(NB)])
            pr = pi = None
            for c in range(NB):
                rr, ii = t1_s[z, c], t2_s[z, c]
                wr, wi = rr - ii, t[c] - rr - ii
                zr, zi = (wr, wi) if c == 0 else (wr + pi, wi - pr)
                pr, pi = wr, wi
                z_s[c, 16 * s:16 * s + 16, :] = jnp.concatenate([zr, zi], axis=0).astype(BF)

        def inv(c):
            z = zeros[3]
            y = (_nn(_ld(dft_v, (), 2 * T, T), _ld(z_s, (c + z,), 0, T))
                 + _nn(_ld(dft_v, (), 3 * T, T), _ld(z_s, (c + z,), T, T)))
            y = y + _ld(kv_s, (), T * c + z, T).astype(F32) * par_s[g, 4][0:1]
            ya_s[g, T * c:T * (c + 1), :] = (_ld(aq_v, (g,), T * c, T).astype(F32) * y).astype(BF)

        for j in range(NB):
            filt(j)
            kv(j)
        for t in range(NQ, NB):
            proj(g, t, zeros[4])
        for s in range(NB):
            slab(s)
        for c in range(NB):
            inv(c)
        return carry

    with _scope("ph_1"):
        lax.fori_loop(0, NG, phase1, 0)
    _start(cp_wo())

    gcolv = g_s[...]
    num_s[0] = jnp.zeros((NQ, D, T), F32)
    for i in range(NQ):
        rden_s[i] = jnp.zeros((H, T), F32)
    mem = [None] * NG
    for s in range(NSEG - 1):
        lhs = []
        for w in range(NG):
            n = _R1[w] - _R0[w]
            vv = jnp.concatenate([v_s[NQ * s + i, _R0[w]:_R1[w], :] for i in range(NQ)], axis=1)
            vv = jnp.concatenate([vv, jnp.ones((8, L), F32)], axis=0)
            upd = _nn(vv, _ld(pk_s, (w,), L * s, L))
            mem[w] = upd if mem[w] is None else mem[w] + upd
            rh = _head_of(lax.broadcasted_iota(I32, (n, T), 0) + _R0[w])
            ch = _head_of(lax.broadcasted_iota(I32, (n, T), 1) + T * w)
            zh = lax.broadcasted_iota(I32, (8, T), 0) + _H0[w]
            ch8 = _head_of(lax.broadcasted_iota(I32, (8, T), 1) + T * w)
            lhs.append(jnp.concatenate([jnp.where(rh == ch, mem[w][:n], 0.0),
                                        jnp.where(zh == ch8, mem[w][n:], 0.0)], axis=0))
        for i in range(NQ):
            t = NQ * (s + 1) + i
            res = [_nn(lhs[w], _ld(pq_s, (t,), T * w, T)) for w in range(NG)]
            den = None
            for w in range(NG):
                lo = _R0[w] if w == 0 else _R1[w - 1]
                hi = _R1[w] if w == NG - 1 else _R0[w + 1]
                num_s[s + 1, i, lo:hi, :] = res[w][lo - _R0[w]:hi - _R0[w]]
                if w + 1 < NG:
                    num_s[s + 1, i, hi:_R1[w], :] = (res[w][hi - _R0[w]:_R1[w] - _R0[w]]
                                                     + res[w + 1][:_R1[w] - hi])
                part = jnp.concatenate(
                    ([jnp.zeros((_H0[w], T), F32)] if _H0[w] else [])
                    + [res[w][_R1[w] - _R0[w]:], jnp.zeros((H - _H0[w], T), F32)], axis=0)[:H]
                den = part if den is None else den + part
            rden_s[t] = gcolv / (den + 1e-6)

    _wait(cp_wo() + cp_conv(NG))
    _start([cp_ya(g) for g in range(NG)])

    tiles = [(i, h, j) for i in cfg["iorder"] for h in range(H) for j in range(i + 1)]

    def segment(s, carry):
        zeros = [zero_s[5 + i] for i in range(2)]
        sub8 = lax.broadcasted_iota(I32, (8, T), 0)
        t0 = pl.multiple_of(s * L, L)
        qws, mx, pvals, acc, fin, held = {}, {}, {}, {}, {}, {}

        def q_weights(i, h):
            f0 = DH * h
            blocks = [jnp.zeros((8, T), U32)] * 8
            for b in (f0 // 16, f0 // 16 + 1):
                blk = q_s.bitcast(U32)[NQ * s + i, 8 * b:8 * b + 8, :]
                lo, hi = f0 // 2 - 8 * b, (f0 + DH) // 2 - 8 * b
                if lo > 0:
                    blk = jnp.where(sub8 >= lo, blk, jnp.uint32(0))
                if hi < 8:
                    blk = jnp.where(sub8 < hi, blk, jnp.uint32(0))
                blocks[b % 8] = blk
            return pltpu.bitcast(jnp.concatenate(blocks, axis=0), BF)

        def stage_a(n):
            i, h, j = tiles[n]
            wb, wa = DH * h // T, (DH * h + DH - 1) // T
            if (i, h) not in qws:
                qws[i, h] = q_weights(i, h)
            kw = _ld(k_s, (wb if wa == wb else NG + wa,), t0 + T * j, T)
            sc = _nn(kw, qws[i, h])
            if i == j:
                sc = sc + mask_s[...]
            m8 = jnp.max(sc.reshape(16, 8, T), axis=0)
            mx[i, h] = m8 if (i, h) not in mx else jnp.maximum(mx[i, h], m8)
            s_ring[n % RING][0] = sc

        def stage_b(n):
            i, h, j = tiles[n]
            if (i, h) not in fin:
                fin[i, h] = jnp.max(mx.pop((i, h)), axis=0, keepdims=True)
            pvals[n] = jnp.exp2(s_ring[n % RING][zeros[0]] - fin[i, h]).astype(BF)

        def stage_c(n):
            i, h, j = tiles[n]
            base = (h // 2) * 2 * DH + (h % 2) * 16
            vv = v_s[NQ * s + j, base:base + 24, :]
            if h % 2 == 0:
                vv = jnp.concatenate([vv[:16], jnp.where(sub8 < 4, vv[16:], 1.0)], axis=0)
            else:
                vv = jnp.concatenate([jnp.where(sub8 >= 4, vv[:8], 1.0), vv[8:]], axis=0)
            o = _nn(vv, pvals.pop(n))
            acc[i, h] = o if j == 0 else acc[i, h] + o
            if j == i:
                a = acc.pop((i, h))
                den = a[DH:DH + 1] if h % 2 == 0 else a[0:1]
                w_dot = (1.0 - g_s[h:h + 1, :]) / den
                w_mem = rden_s[NQ * s + i, h:h + 1, :]
                o = a * w_dot + num_s[s, i, base:base + 24, :] * w_mem
                if h % 2 == 0:
                    ot_s[i][0, base:base + 16, :] = o[:16]
                    held[i] = o[16:]
                else:
                    mid = jnp.where(sub8 < 4, held.pop(i), o[:8])
                    ot_s[i][0, base:base + 24, :] = jnp.concatenate([mid, o[8:]], axis=0)

        def out_proj(i):
            ot = jnp.concatenate([ot_s[i][zeros[1], T * w:T * (w + 1), :].T for w in range(NG)], axis=1)
            wo = jnp.concatenate([_ld(wo_v, (c,), 0, D) for c in range(NG)], axis=1)
            yb_s[s, T * i:T * (i + 1), :] = _nn(ot.astype(BF), wo).astype(BF)

        n = len(tiles)
        lb, lc, grp = cfg["lagB"], cfg["lagC"], cfg["G"]
        last = {i: max(k for k in range(n) if tiles[k][0] == i) for i in cfg["iorder"]}
        todo = list(cfg["iorder"])
        for tt in range(0, n + lb + lc, grp):
            for k in range(tt, tt + grp):
                if k < n:
                    stage_a(k)
            for k in range(tt, tt + grp):
                if 0 <= k - lb < n:
                    stage_b(k - lb)
            for k in range(tt, tt + grp):
                if 0 <= k - lb - lc < n:
                    stage_c(k - lb - lc)
            if len(todo) > 2 and tt - lb - lc > last[todo[0]] + cfg["olag"]:
                out_proj(todo.pop(0))
            if len(todo) == 2 and tt + grp >= n:
                out_proj(todo.pop(0))
        for i in todo:
            out_proj(i)
        cp_yb(s).start()
        return carry

    with _scope("ph_2"):
        lax.fori_loop(0, NSEG, segment, 0) if cfg['p2'] == 1 else [cp_yb(s).start() for s in range(NSEG)]

    with _scope("ph_tail"):
        for g in range(NG):
            cp_ya(g).wait()
        for s in range(NSEG):
            cp_yb(s).wait()


@jax.jit
def pallas_concat_heads__ssm_conv_h3__memory_aug_infini_attn__prompt_kernel(
    A_q, A_k, A_v, A_shift_k, A_ssm_k, A_ssm_D, B_x, B_wq, B_wk, B_wv, B_wo, B_beta,
):
    scratch = [
        pltpu.VMEM((NG + 1, S, T), BF),
        pltpu.VMEM((NG + 1, S, T), BF),
        pltpu.VMEM((NG + 1, S, T), BF),
        pltpu.VMEM((NG + 1, T, S), BF),
        pltpu.VMEM((NG, S, T), BF),
        pltpu.VMEM((NG, D, T), BF),
        pltpu.VMEM((NG, D, T), BF),
        pltpu.VMEM((NG, D, T), BF),
        pltpu.VMEM((NG, D, T), BF),
        pltpu.VMEM((4, D), BF),
        pltpu.VMEM((D,), BF),
        pltpu.VMEM((H,), BF),
        pltpu.VMEM((4 * T, T), BF),
        pltpu.VMEM((NG, NG, 2 * T, T), BF),
        pltpu.VMEM((S, T), BF),
        pltpu.VMEM((NB, 2 * T, T), F32),
        pltpu.VMEM((NB, 2 * T, T), F32),
        pltpu.VMEM((NB, 2 * T, T), BF),
        pltpu.VMEM((NG, S, T), BF),
        pltpu.VMEM((2 * NG, S, T), BF),
        pltpu.VMEM((NB, D, T), BF),
        pltpu.VMEM((NB, D, T), F32),
        pltpu.VMEM((NG, S, T), BF),
        pltpu.VMEM((NB, D, T), BF),
        pltpu.VMEM((NSEG, NQ, D, T), F32),
        pltpu.VMEM((NB, H, T), F32),
        pltpu.VMEM((NSEG, L, D), BF),
        pltpu.VMEM((T, T), F32),
        pltpu.VMEM((NG, 5, 8, T), F32),
        pltpu.VMEM((H, T), F32),
        pltpu.SMEM((8,), I32),
        pltpu.SemaphoreType.DMA((2 + NSEG,)),
        pltpu.SemaphoreType.DMA((4 * NG + 3,)),
        pltpu.SemaphoreType.DMA((NG + NSEG,)),
        *[pltpu.VMEM((1, D, T), F32)] * NQ,
        *[pltpu.VMEM((1, T, T), F32)] * RING,
        *[pltpu.VMEM((1, NB, 8, T), F32)] * (2 * CFG['tr']),
    ]
    hbm = pl.BlockSpec(memory_space=pl.ANY)
    out = pl.pallas_call(
        _kernel,
        out_shape=jax.ShapeDtypeStruct((S, 2 * D), BF),
        in_specs=[hbm] * 13,
        out_specs=hbm,
        scratch_shapes=scratch,
        compiler_params=pltpu.CompilerParams(vmem_limit_bytes=100 * 1024 * 1024),
        name="h3_infini",
    )(A_q.reshape(S, D), A_k.reshape(S, D), A_v.reshape(S, D), A_shift_k.T, A_ssm_k, A_ssm_D,
      B_x.reshape(S, D), B_wq, B_wk, B_wv, B_wo, B_beta, _DFT)
    return out.reshape(1, S, 2 * D)
```

```python
import jax
import jax.numpy as jnp
import numpy as np
from jax import lax
import jax.experimental.pallas as pl
import jax.experimental.pallas.tpu as pltpu

BF = jnp.bfloat16
F32 = jnp.float32
U32 = jnp.uint32
I32 = jnp.int32

S = 2048
D = 640
H = 32
DH = 20
NSEG = 4
L = S // NSEG
T = 128
NB = S // T
NQ = L // T
NG = D // T
RING = 24
LOG2E = 1.4426950408889634
QSCALE = DH ** -0.5 * LOG2E
NEG = -1e9 * LOG2E

def _ident(d):
    return d


def _front(*names):
    return lambda d: {**{k: d[k] for k in d if k.startswith(names)}, **d}


CFG = dict(perm=_ident, dm=2, fill=0, n=4, ord=0, npre=5, lead=1, pre=((0,), (1,), (2, 3, 4)), merge=0, tr=4, parts='', fu=1, xw=2, wt0=1, p2=1, lagB=16, lagC=4, G=4, iorder=(0, 1, 2, 3), olag=8, inv_at=16, slabs=[1] * 16, scopes=False)


def _dft_matrices():
    theta = (0.5 * np.pi + 2.0 * np.pi * np.arange(T)) / T
    ang = theta[:, None] * np.arange(T)[None, :]
    f = np.stack([np.cos(ang).reshape(NB, 8, T), np.sin(ang).reshape(NB, 8, T)], axis=1)
    f = f.reshape(2 * T, T)
    g = (f.T / T).reshape(T, 2, T).transpose(1, 0, 2).reshape(2 * T, T)
    return np.concatenate([f, g], axis=0).astype(BF)


_DFT = _dft_matrices()

_H0 = [(T * w) // DH for w in range(NG)]
_H1 = [(T * w + T - 1) // DH for w in range(NG)]
_R0 = [(DH * h) // 8 * 8 for h in _H0]
_R1 = [-(-(DH * (h + 1)) // 8) * 8 for h in _H1]


def _phi(t):
    return jnp.where(t > 0, t + 1.0, jnp.exp(t))


def _head_of(idx):
    return (idx * 3277) >> 16


def _ld(ref, idx, r0, n):
    if isinstance(r0, int):
        rows = pl.ds(r0 // 2, n // 2)
    else:
        rows = pl.ds(pl.multiple_of(r0 // 2, 8), n // 2)
    return pltpu.bitcast(ref.bitcast(U32)[(*idx, rows, slice(None))], BF)


def _nn(a, b):
    return lax.dot_general(a, b, (((1,), (0,)), ((), ())), preferred_element_type=F32)


def _nt(a, b):
    return lax.dot_general(a, b, (((1,), (1,)), ((), ())), preferred_element_type=F32)


def _short_conv(us, ks):
    out = []
    for c in range(NB):
        acc = us[c] * ks[0]
        for j in range(1, c + 1):
            acc = acc + us[c - j] * ks[j]
        out.append(acc)
    return out


def _start(copies, priority=0):
    for c in copies:
        c.start(priority=priority)


def _wait(copies):
    for c in copies:
        c.wait()


def _scope(name):
    return jax.named_scope(name) if CFG["scopes"] else _NoScope()


class _NoScope:
    def __enter__(self):
        return None

    def __exit__(self, *exc):
        return False


def _scratch():
    vm = pltpu.VMEM
    return dict(
        wo_v=vm((NG, D, T), BF),
        k_s=vm((2 * NG, S, T), BF),
        q_s=vm((NB, D, T), BF),
        v_s=vm((NB, D, T), F32),
        num_s=vm((NSEG, NQ, D, T), F32),
        rden_s=vm((NB, H, T), F32),
        yb_s=vm((NSEG, L, D), BF),
        mask_s=vm((T, T), F32),
        g_s=vm((H, T), F32),
        **{f"ot{i}": vm((1, D, T), F32) for i in range(NQ)},
        **{f"sr{i}": vm((1, T, T), F32) for i in range(RING)},
        aq_v=vm((NG + 2, S, T), BF),
        ak_v=vm((NG + 2, S, T), BF),
        av_v=vm((NG + 2, S, T), BF),
        fk_v=vm((NG + 2, T, S), BF),
        x_v=vm((NG, S, T), BF),
        wq_v=vm((NG, D, T), BF),
        wk_v=vm((NG, D, T), BF),
        wv_v=vm((NG, D, T), BF),
        dft_v=vm((4 * T, T), BF),
        wt_s=vm((NG, NG, 2 * T, T), BF),
        kv_s=vm((S, T), BF),
        uf_s=vm((NB, 2 * T, T), F32),
        kf_s=vm((NB, 2 * T, T), F32),
        z_s=vm((NB, 2 * T, T), BF),
        ya_s=vm((NG, S, T), BF),
        pk_s=vm((NG, S, T), BF),
        pq_s=vm((NB, D, T), BF),
        par_s=vm((NG, 5, 8, T), F32),
        **{f"tr{i}": vm((1, NB, 8, T), F32) for i in range(8)},
        sk_v=vm((4, D), BF),
        dd_v=vm((D,), BF),
        beta_v=vm((H,), BF),
        zero_s=pltpu.SMEM((8,), I32),
        sem_s=pltpu.SemaphoreType.DMA((4 + 2 * NG,)),
        sem_g=pltpu.SemaphoreType.DMA((NG + 2,)),
        sem_out=pltpu.SemaphoreType.DMA((NG + 2 * NSEG,)),
    )


def _kernel(aq_hbm, ak_hbm, av_hbm, sk_hbm, fk_hbm, dd_hbm, x_hbm, wq_hbm, wk_hbm, wv_hbm,
            wo_hbm, beta_hbm, dft_hbm, out_hbm, *, aq_v, ak_v, av_v, fk_v, x_v, wq_v, wk_v, wv_v,
            wo_v, sk_v, dd_v, beta_v, dft_v, wt_s, kv_s, uf_s, kf_s, z_s, ya_s, k_s, q_s, v_s,
            pk_s, pq_s, num_s, rden_s, yb_s, mask_s, par_s, g_s, zero_s, sem_s, sem_g, sem_out,
            **rings):
    cfg = CFG
    ot_s = [rings[f"ot{i}"] for i in range(NQ)]
    s_ring = [rings[f"sr{i}"] for i in range(RING)]
    t_ring = [rings[f"tr{i}"] for i in range(8)]

    def col(g):
        return pl.ds(g * T if isinstance(g, int) else pl.multiple_of(g * T, T), T)

    def cp_small():
        return [pltpu.make_async_copy(src, dst, sem_s.at[0]) for src, dst in
                ((sk_hbm, sk_v), (dd_hbm, dd_v), (beta_hbm, beta_v), (dft_hbm, dft_v))]

    def cp_x(c):
        rows = pl.ds(0, PRE) if c == 0 else pl.ds(PRE, S - PRE)
        return [pltpu.make_async_copy(x_hbm.at[rows, col(w)], x_v.at[w, rows], sem_s.at[1 + c])
                for w in range(NG)]

    def cp_wo():
        return [pltpu.make_async_copy(wo_hbm.at[:, col(w)], wo_v.at[w], sem_s.at[3])
                for w in range(NG)]

    def src_group(g):
        return min(g, NG - 1) if isinstance(g, int) else jnp.minimum(g, NG - 1)

    def cp_conv(g):
        src = src_group(g)
        return [pltpu.make_async_copy(fk_hbm.at[col(src), :], fk_v.at[g], sem_g.at[g])] + [
            pltpu.make_async_copy(a.at[:, col(src)], dst.at[g], sem_g.at[g])
            for a, dst in ((ak_hbm, ak_v), (av_hbm, av_v), (aq_hbm, aq_v))]

    def cp_wk(g):
        return [pltpu.make_async_copy(wk_hbm.at[:, col(g)], wk_v.at[g], sem_s.at[4 + g])]

    def cp_wqv(g):
        return [pltpu.make_async_copy(src.at[:, col(g)], dst.at[g], sem_s.at[4 + NG + g])
                for src, dst in ((wq_hbm, wq_v), (wv_hbm, wv_v))]

    def cp_w(windows):
        return [c for g in windows for c in cp_wk(g) + cp_wqv(g)]

    def cp_ya(g):
        return pltpu.make_async_copy(ya_s.at[g], out_hbm.at[:, col(g)], sem_out.at[g])

    def cp_yb(s, part):
        lo, n = ((0, L - T), (L - T, T))[part]
        r0 = s * L + lo if isinstance(s, int) else pl.multiple_of(s * L + lo, T)
        return pltpu.make_async_copy(yb_s.at[s, pl.ds(lo, n)], out_hbm.at[pl.ds(r0, n), D:2 * D],
                                     sem_out.at[NG + 2 * s + part])

    PRE = T * cfg["npre"]
    steps = cfg["pre"]
    _start(cp_x(0) + cp_w(steps[0]))
    _start(cp_x(1) + cp_conv(0), priority=1)

    for i in range(8):
        zero_s[i] = 0
    r_i = lax.broadcasted_iota(I32, (T, T), 0)
    c_i = lax.broadcasted_iota(I32, (T, T), 1)
    mask_s[...] = jnp.where(r_i <= c_i, 0.0, NEG)

    def x_tile(t):
        return jnp.concatenate([_ld(x_v, (c,), T * t, T) for c in range(NG)], axis=1)

    def transpose_w(g):
        for c in range(NG):
            wt_s[g, c, 0:T, :] = _ld(wq_v, (g,), T * c, T).T
            wt_s[g, c, T:2 * T, :] = _ld(wv_v, (g,), T * c, T).T

    def proj_k(g, t, z):
        rows = slice(T * t, T * (t + 1))
        words = slice(T * t // 2, T * (t + 1) // 2)
        k = _nn(x_tile(t), _ld(wk_v, (g,), 0, D))
        k_s[g, rows, :] = k.astype(BF)
        pk_s[g, rows, :] = _phi(k).astype(BF)
        if not isinstance(g, int) or g:
            gp = g - 1 if isinstance(g, int) else jnp.maximum(g - 1, 0)
            ku = k_s.bitcast(U32)
            ku[NG + g, words, :] = jnp.where(c_i[:T // 2] < 64, ku[g + z, words, :], ku[gp + z, words, :])

    def proj_qv(g, t, z):
        wt = jnp.concatenate([_ld(wt_s, (g + z, c), 0, 2 * T) for c in range(NG)], axis=1)
        qv = _nt(wt, x_tile(t))
        q = qv[:T]
        q_s[t, col(g), :] = (q * QSCALE).astype(BF)
        pq_s[t, col(g), :] = _phi(q).astype(BF)
        v_s[t, col(g), :] = qv[T:]

    with _scope("ph_wait0"):
        _wait(cp_x(0) + cp_w(steps[0]))
    with _scope("ph_10"):
        z0 = zero_s[0]
        num_s[0] = jnp.zeros((NQ, D, T), F32)
        rden_s[0:NQ] = jnp.zeros((NQ, H, T), F32)
        for n, windows in enumerate(steps):
            if n + 1 < len(steps):
                _start(cp_w(steps[n + 1]) + (cp_small() if n == 0 else []))
            if n:
                _wait(cp_w(windows))
            if n == len(steps) - 1:
                _wait(cp_small())
            taps = sk_v[...].astype(F32)
            dvec = dd_v[...].astype(F32).reshape(1, D)
            for g in range(NG):
                for j in range(4):
                    par_s[g, j] = jnp.broadcast_to(taps[j:j + 1, T * g:T * (g + 1)], (8, T))
                par_s[g, 4] = jnp.broadcast_to(dvec[:, T * g:T * (g + 1)], (8, T))
            gate = jax.nn.sigmoid(beta_v[...].astype(F32).reshape(1, H)).astype(BF).astype(F32)
            hr = lax.broadcasted_iota(I32, (H, H), 0)
            hc = lax.broadcasted_iota(I32, (H, H), 1)
            gcol = jnp.sum(jnp.where(hr == hc, jnp.broadcast_to(gate, (H, H)), 0.0), axis=1, keepdims=True)
            g_s[...] = jnp.broadcast_to(gcol, (H, T))
            for g in windows:
                transpose_w(g)
            for fn in (proj_k, proj_qv):
                for g in windows:
                    for t in range(cfg["npre"]):
                        fn(g, t, z0)

        _wait(cp_x(1) + cp_conv(0))
        _start(cp_conv(1))
        _start(cp_wo(), priority=1)

    def phase1(g, carry):
        zeros = [zero_s[i] for i in range(5)]
        fwd = lambda: _ld(dft_v, (), 0, 2 * T)

        def filt(j):
            kf_s[j] = _nt(fwd(), fk_v[g, :, T * j:T * (j + 1)])

        def kv(a):
            cur = _ld(ak_v, (g,), T * a, T).astype(F32)
            if a == 0:
                prev = jnp.zeros((8, T), F32)
            else:
                prev = _ld(ak_v, (g,), T * a - 16, 16).astype(F32)[8:]
            ext = jnp.concatenate([prev, cur], axis=0)
            acc = cur * par_s[g, 0][0:1]
            for j in range(1, 4):
                acc = acc + ext[8 - j:8 - j + T] * par_s[g, j][0:1]
            u = (acc * _ld(av_v, (g,), T * a, T).astype(F32)).astype(BF)
            kv_s[T * a:T * (a + 1), :] = u
            uf_s[a] = _nn(fwd(), u)

        def slab(s):
            re, im = slice(16 * s, 16 * s + 8), slice(16 * s + 8, 16 * s + 16)
            t1_s, t2_s = t_ring[2 * (s % cfg['tr'])], t_ring[2 * (s % cfg['tr']) + 1]
            for part, dst, z in ((re, t1_s, zeros[0]), (im, t2_s, zeros[1])):
                t = _short_conv([uf_s[a + z, part, :] for a in range(NB)],
                                [kf_s[j + z, part, :] for j in range(NB)])
                for c in range(NB):
                    dst[0, c] = t[c]
            z = zeros[2]
            t = _short_conv([uf_s[a + z, re, :] + uf_s[a + z, im, :] for a in range(NB)],
                            [kf_s[j + z, re, :] + kf_s[j + z, im, :] for j in range(NB)])
            pr = pi = None
            for c in range(NB):
                rr, ii = t1_s[z, c], t2_s[z, c]
                wr, wi = rr - ii, t[c] - rr - ii
                zr, zi = (wr, wi) if c == 0 else (wr + pi, wi - pr)
                pr, pi = wr, wi
                z_s[c, 16 * s:16 * s + 16, :] = jnp.concatenate([zr, zi], axis=0).astype(BF)

        def inv(c):
            z = zeros[3]
            y = (_nn(_ld(dft_v, (), 2 * T, T), _ld(z_s, (c + z,), 0, T))
                 + _nn(_ld(dft_v, (), 3 * T, T), _ld(z_s, (c + z,), T, T)))
            y = y + _ld(kv_s, (), T * c + z, T).astype(F32) * par_s[g, 4][0:1]
            ya_s[g, T * c:T * (c + 1), :] = (_ld(aq_v, (g,), T * c, T).astype(F32) * y).astype(BF)

        lead = cfg["lead"]
        for j in range(NB + lead):
            if j < NB:
                filt(j)
            if j >= lead:
                kv(j - lead)
        if cfg["ord"] == 0:
            for t in range(cfg["npre"], NB):
                proj_k(g, t, zeros[4])
                proj_qv(g, t, zeros[4])
            for s in range(NB):
                slab(s)
        elif cfg["ord"] == 1:
            for s in range(NB):
                slab(s)
            for t in range(cfg["npre"], NB):
                proj_k(g, t, zeros[4])
                proj_qv(g, t, zeros[4])
        else:
            nt = NB - cfg["npre"]
            for n in range(nt):
                proj_k(g, cfg["npre"] + n, zeros[4])
                proj_qv(g, cfg["npre"] + n, zeros[4])
                for s in range(NB * n // nt, NB * (n + 1) // nt):
                    slab(s)
        for c in range(NB):
            inv(c)
        _start(cp_conv(g + 2))
        _wait(cp_conv(g + 1))
        return carry

    with _scope("ph_1"):
        lax.fori_loop(0, NG, phase1, 0)

    gcolv = g_s[...]
    mem = [None] * NG
    for s in range(NSEG - 1):
        lhs = []
        for w in range(NG):
            n = _R1[w] - _R0[w]
            vv = jnp.concatenate([v_s[NQ * s + i, _R0[w]:_R1[w], :] for i in range(NQ)], axis=1)
            vv = jnp.concatenate([vv, jnp.ones((8, L), F32)], axis=0)
            upd = _nn(vv, _ld(pk_s, (w,), L * s, L))
            mem[w] = upd if mem[w] is None else mem[w] + upd
            rh = _head_of(lax.broadcasted_iota(I32, (n, T), 0) + _R0[w])
            ch = _head_of(lax.broadcasted_iota(I32, (n, T), 1) + T * w)
            zh = lax.broadcasted_iota(I32, (8, T), 0) + _H0[w]
            ch8 = _head_of(lax.broadcasted_iota(I32, (8, T), 1) + T * w)
            lhs.append(jnp.concatenate([jnp.where(rh == ch, mem[w][:n], 0.0),
                                        jnp.where(zh == ch8, mem[w][n:], 0.0)], axis=0))
        for i in range(NQ):
            t = NQ * (s + 1) + i
            res = [_nn(lhs[w], _ld(pq_s, (t,), T * w, T)) for w in range(NG)]
            den = None
            for w in range(NG):
                lo = _R0[w] if w == 0 else _R1[w - 1]
                hi = _R1[w] if w == NG - 1 else _R0[w + 1]
                num_s[s + 1, i, lo:hi, :] = res[w][lo - _R0[w]:hi - _R0[w]]
                if w + 1 < NG:
                    num_s[s + 1, i, hi:_R1[w], :] = (res[w][hi - _R0[w]:_R1[w] - _R0[w]]
                                                     + res[w + 1][:_R1[w] - hi])
                part = jnp.concatenate(
                    ([jnp.zeros((_H0[w], T), F32)] if _H0[w] else [])
                    + [res[w][_R1[w] - _R0[w]:], jnp.zeros((H - _H0[w], T), F32)], axis=0)[:H]
                den = part if den is None else den + part
            rden_s[t] = gcolv / (den + 1e-6)

    _wait(cp_wo())
    _start([cp_ya(g) for g in range(NG)])

    tiles = [(i, h, j) for i in cfg["iorder"] for h in range(H) for j in range(i + 1)]

    def segment(s, carry):
        zeros = [zero_s[5 + i] for i in range(2)]
        sub8 = lax.broadcasted_iota(I32, (8, T), 0)
        t0 = pl.multiple_of(s * L, L)
        qws, mx, pvals, acc, fin, held = {}, {}, {}, {}, {}, {}

        def q_weights(i, h):
            f0 = DH * h
            blocks = [jnp.zeros((8, T), U32)] * 8
            for b in (f0 // 16, f0 // 16 + 1):
                blk = q_s.bitcast(U32)[NQ * s + i, 8 * b:8 * b + 8, :]
                lo, hi = f0 // 2 - 8 * b, (f0 + DH) // 2 - 8 * b
                if lo > 0:
                    blk = jnp.where(sub8 >= lo, blk, jnp.uint32(0))
                if hi < 8:
                    blk = jnp.where(sub8 < hi, blk, jnp.uint32(0))
                blocks[b % 8] = blk
            return pltpu.bitcast(jnp.concatenate(blocks, axis=0), BF)

        def q_shared(i, m):
            f0 = 2 * DH * m
            low = lax.broadcasted_iota(I32, (8, T), 1) < 64
            blocks = [jnp.zeros((8, T), U32)] * 8
            for b in range(f0 // 16, (f0 + 2 * DH - 1) // 16 + 1):
                blk = q_s.bitcast(U32)[NQ * s + i, 8 * b:8 * b + 8, :]
                row = sub8 + 8 * b - f0 // 2
                in_a = (row >= 0) & (row < DH // 2) & low
                in_b = (row >= DH // 2) & (row < DH) & jnp.logical_not(low)
                blocks[b % 8] = jnp.where(in_a, pltpu.roll(blk, 64, 1), jnp.where(in_b, blk, jnp.uint32(0)))
            return pltpu.bitcast(jnp.concatenate(blocks, axis=0), BF)

        def keep(n, r0, sc):
            i, h, _ = tiles[n]
            m8 = jnp.max(sc.reshape(sc.shape[0] // 8, 8, T), axis=0)
            mx[i, h] = m8 if (i, h) not in mx else jnp.maximum(mx[i, h], m8)
            s_ring[n % RING][0, r0:r0 + sc.shape[0], :] = sc

        def stage_a(n):
            i, h, j = tiles[n]
            f0 = 2 * DH * (h // 2)
            wb, wa = f0 // T, (f0 + 2 * DH - 1) // T
            win = (wb if wa == wb else NG + wa,)
            if (i, h) not in qws:
                qws[i, h] = q_weights(i, h)
            merge = cfg["merge"] and i > 0
            if merge and j == i - 1:
                sc = _nn(_ld(k_s, win, t0 + T * j, T + 64), qws[i, h])
                keep(n, 0, sc[:T])
                keep(n + 1, 0, sc[T:] + mask_s[0:64, :])
            elif j < i:
                keep(n, 0, _nn(_ld(k_s, win, t0 + T * j, T), qws[i, h]))
            else:
                if not merge:
                    keep(n, 0, _nn(_ld(k_s, win, t0 + T * j, 64), qws[i, h]) + mask_s[0:64, :])
                if h % 2 == 0:
                    sh = _nn(_ld(k_s, win, t0 + T * j + 64, 64), q_shared(i, h // 2))
                    keep(n, 64, pltpu.roll(sh, 64, 1) + mask_s[64:T, :])
                    keep(n + i + 1, 64, sh + mask_s[64:T, :])

        def stage_b(n):
            i, h, j = tiles[n]
            if (i, h) not in fin:
                fin[i, h] = jnp.max(mx.pop((i, h)), axis=0, keepdims=True)
            pvals[n] = jnp.exp2(s_ring[n % RING][zeros[0]] - fin[i, h]).astype(BF)

        def stage_c(n):
            i, h, j = tiles[n]
            base = (h // 2) * 2 * DH + (h % 2) * 16
            vv = v_s[NQ * s + j, base:base + 24, :]
            if h % 2 == 0:
                vv = jnp.concatenate([vv[:16], jnp.where(sub8 < 4, vv[16:], 1.0)], axis=0)
            else:
                vv = jnp.concatenate([jnp.where(sub8 >= 4, vv[:8], 1.0), vv[8:]], axis=0)
            o = _nn(vv, pvals.pop(n))
            acc[i, h] = o if j == 0 else acc[i, h] + o
            if j == i:
                a = acc.pop((i, h))
                den = a[DH:DH + 1] if h % 2 == 0 else a[0:1]
                w_dot = (1.0 - g_s[h:h + 1, :]) / den
                w_mem = rden_s[NQ * s + i, h:h + 1, :]
                o = a * w_dot + num_s[s, i, base:base + 24, :] * w_mem
                if h % 2 == 0:
                    ot_s[i][0, base:base + 16, :] = o[:16]
                    held[i] = o[16:]
                else:
                    mid = jnp.where(sub8 < 4, held.pop(i), o[:8])
                    ot_s[i][0, base:base + 24, :] = jnp.concatenate([mid, o[8:]], axis=0)

        def out_proj(i):
            ot = jnp.concatenate([ot_s[i][zeros[1], T * w:T * (w + 1), :].T for w in range(NG)], axis=1)
            wo = jnp.concatenate([_ld(wo_v, (c,), 0, D) for c in range(NG)], axis=1)
            yb_s[s, T * i:T * (i + 1), :] = _nn(ot.astype(BF), wo).astype(BF)

        n = len(tiles)
        lb, lc, grp = cfg["lagB"], cfg["lagC"], cfg["G"]
        last = {i: max(k for k in range(n) if tiles[k][0] == i) for i in cfg["iorder"]}
        todo = list(cfg["iorder"])
        for tt in range(0, n + lb + lc, grp):
            for k in range(tt, tt + grp):
                if k < n:
                    stage_a(k)
            for k in range(tt, tt + grp):
                if 0 <= k - lb < n:
                    stage_b(k - lb)
            for k in range(tt, tt + grp):
                if 0 <= k - lb - lc < n:
                    stage_c(k - lb - lc)
            if len(todo) > 3 and tt - lb - lc > last[todo[0]] + cfg["olag"]:
                out_proj(todo.pop(0))
            if len(todo) == 3 and tt + grp >= n:
                out_proj(todo.pop(0))
        for i in todo:
            if i == NQ - 1:
                cp_yb(s, 0).start()
            out_proj(i)
        cp_yb(s, 1).start()
        return carry

    with _scope("ph_2"):
        lax.fori_loop(0, cfg['n'], lambda q, c: segment(q & 3, c), 0)

    with _scope("ph_tail"):
        _wait(cp_conv(NG + 1))
        for g in range(NG):
            cp_ya(g).wait()
        for s in range(cfg['n']):
            cp_yb(s & 3, 0).wait()
            cp_yb(s & 3, 1).wait()


@jax.jit
def pallas_concat_heads__ssm_conv_h3__memory_aug_infini_attn__prompt_kernel(
    A_q, A_k, A_v, A_shift_k, A_ssm_k, A_ssm_D, B_x, B_wq, B_wk, B_wv, B_wo, B_beta,
):
    hbm = pl.BlockSpec(memory_space=pl.ANY)
    scratch = CFG['perm'](_scratch())

    def body(*refs):
        _kernel(*refs[:14], **dict(zip(scratch, refs[14:])))

    out = pl.pallas_call(
        body,
        out_shape=jax.ShapeDtypeStruct((S, 2 * D), BF),
        in_specs=[hbm] * 13,
        out_specs=hbm,
        scratch_shapes=list(scratch.values()),
        compiler_params=pltpu.CompilerParams(vmem_limit_bytes=100 * 1024 * 1024),
        name="h3_infini",
    )(A_q.reshape(S, D), A_k.reshape(S, D), A_v.reshape(S, D), A_shift_k.T, A_ssm_k, A_ssm_D,
      B_x.reshape(S, D), B_wq, B_wk, B_wv, B_wo, B_beta, _DFT)
    return out.reshape(1, S, 2 * D)
```

```python
import jax
import jax.numpy as jnp
import numpy as np
from jax import lax
import jax.experimental.pallas as pl
import jax.experimental.pallas.tpu as pltpu

BF = jnp.bfloat16
F32 = jnp.float32
U32 = jnp.uint32
I32 = jnp.int32

S = 2048
D = 640
H = 32
DH = 20
NSEG = 4
L = S // NSEG
T = 128
NB = S // T
NQ = L // T
NG = D // T
RING = 24
LOG2E = 1.4426950408889634
QSCALE = DH ** -0.5 * LOG2E
NEG = -1e9 * LOG2E

def _ident(d):
    return d


def _front(*names):
    return lambda d: {**{k: d[k] for k in d if k.startswith(names)}, **d}


CFG = dict(nhead=2, early=0, perm=_ident, dm=2, fill=0, n=4, xlag=1, npre=5, lead=1, pre=((0,), (1,), (2, 3, 4)), merge=0, tr=4, parts='', fu=1, xw=2, wt0=1, p2=1, lagB=16, lagC=4, G=4, iorder=(0, 1, 2, 3), olag=8, inv_at=16, slabs=[1] * 16, scopes=False)


def _dft_matrices():
    theta = (0.5 * np.pi + 2.0 * np.pi * np.arange(T)) / T
    ang = theta[:, None] * np.arange(T)[None, :]
    f = np.stack([np.cos(ang).reshape(NB, 8, T), np.sin(ang).reshape(NB, 8, T)], axis=1)
    f = f.reshape(2 * T, T)
    g = (f.T / T).reshape(T, 2, T).transpose(1, 0, 2).reshape(2 * T, T)
    return np.concatenate([f, g], axis=0).astype(BF)


_DFT = _dft_matrices()

_H0 = [(T * w) // DH for w in range(NG)]
_H1 = [(T * w + T - 1) // DH for w in range(NG)]
_R0 = [(DH * h) // 8 * 8 for h in _H0]
_R1 = [-(-(DH * (h + 1)) // 8) * 8 for h in _H1]


def _phi(t):
    return jnp.where(t > 0, t + 1.0, jnp.exp(t))


def _head_of(idx):
    return (idx * 3277) >> 16


def _ld(ref, idx, r0, n):
    if isinstance(r0, int):
        rows = pl.ds(r0 // 2, n // 2)
    else:
        rows = pl.ds(pl.multiple_of(r0 // 2, 8), n // 2)
    return pltpu.bitcast(ref.bitcast(U32)[(*idx, rows, slice(None))], BF)


def _nn(a, b):
    return lax.dot_general(a, b, (((1,), (0,)), ((), ())), preferred_element_type=F32)


def _nt(a, b):
    return lax.dot_general(a, b, (((1,), (1,)), ((), ())), preferred_element_type=F32)


def _short_conv(us, ks):
    out = []
    for c in range(NB):
        acc = us[c] * ks[0]
        for j in range(1, c + 1):
            acc = acc + us[c - j] * ks[j]
        out.append(acc)
    return out


def _start(copies, priority=0):
    for c in copies:
        c.start(priority=priority)


def _wait(copies):
    for c in copies:
        c.wait()


def _scope(name):
    return jax.named_scope(name) if CFG["scopes"] else _NoScope()


class _NoScope:
    def __enter__(self):
        return None

    def __exit__(self, *exc):
        return False


def _scratch():
    vm = pltpu.VMEM
    return dict(
        wo_v=vm((NG, D, T), BF),
        k_s=vm((2 * NG, S, T), BF),
        q_s=vm((NB, D, T), BF),
        v_s=vm((NB, D, T), F32),
        num_s=vm((NSEG, NQ, D, T), F32),
        rden_s=vm((NB, H, T), F32),
        yb_s=vm((NSEG, L, D), BF),
        mask_s=vm((T, T), F32),
        g_s=vm((H, T), F32),
        **{f"ot{i}": vm((1, D, T), F32) for i in range(NQ)},
        **{f"sr{i}": vm((1, T, T), F32) for i in range(RING)},
        aq_v=vm((NG + 2, S, T), BF),
        ak_v=vm((NG + 2, S, T), BF),
        av_v=vm((NG + 2, S, T), BF),
        fk_v=vm((NG + 2, T, S), BF),
        x_v=vm((NG, S, T), BF),
        wq_v=vm((NG, D, T), BF),
        wk_v=vm((NG, D, T), BF),
        wv_v=vm((NG, D, T), BF),
        dft_v=vm((4 * T, T), BF),
        wt_s=vm((NG, NG, 2 * T, T), BF),
        kv_s=vm((S, T), BF),
        uf_s=vm((NB, 2 * T, T), F32),
        kf_s=vm((NB, 2 * T, T), F32),
        z_s=vm((NB, 2 * T, T), BF),
        ya_s=vm((NG, S, T), BF),
        pk_s=vm((NG, S, T), BF),
        pq_s=vm((NB, D, T), BF),
        par_s=vm((NG, 5, 8, T), F32),
        **{f"tr{i}": vm((1, NB, 8, T), F32) for i in range(8)},
        sk_v=vm((4, D), BF),
        dd_v=vm((D,), BF),
        beta_v=vm((H,), BF),
        zero_s=pltpu.SMEM((8,), I32),
        sem_s=pltpu.SemaphoreType.DMA((4 + 2 * NG,)),
        sem_g=pltpu.SemaphoreType.DMA((NG + 2,)),
        sem_x=pltpu.SemaphoreType.DMA((2,)),
        sem_out=pltpu.SemaphoreType.DMA((NG + 2 * NSEG,)),
    )


def _kernel(aq_hbm, ak_hbm, av_hbm, sk_hbm, fk_hbm, dd_hbm, x_hbm, wq_hbm, wk_hbm, wv_hbm,
            wo_hbm, beta_hbm, dft_hbm, out_hbm, *, aq_v, ak_v, av_v, fk_v, x_v, wq_v, wk_v, wv_v,
            wo_v, sk_v, dd_v, beta_v, dft_v, wt_s, kv_s, uf_s, kf_s, z_s, ya_s, k_s, q_s, v_s,
            pk_s, pq_s, num_s, rden_s, yb_s, mask_s, par_s, g_s, zero_s, sem_s, sem_g, sem_x, sem_out,
            **rings):
    cfg = CFG
    ot_s = [rings[f"ot{i}"] for i in range(NQ)]
    s_ring = [rings[f"sr{i}"] for i in range(RING)]
    t_ring = [rings[f"tr{i}"] for i in range(8)]

    def col(g):
        return pl.ds(g * T if isinstance(g, int) else pl.multiple_of(g * T, T), T)

    def cp_small():
        return [pltpu.make_async_copy(src, dst, sem_s.at[0]) for src, dst in
                ((sk_hbm, sk_v), (dd_hbm, dd_v), (beta_hbm, beta_v), (dft_hbm, dft_v))]

    def cp_x(c):
        lo, hi = ((0, PRE), (PRE, NB))[c]
        rows = pl.ds(T * lo, T * (hi - lo))
        return [pltpu.make_async_copy(x_hbm.at[rows, col(w)], x_v.at[w, rows], sem_x.at[c])
                for w in range(NG)]

    def cp_wo():
        return [pltpu.make_async_copy(wo_hbm.at[:, col(w)], wo_v.at[w], sem_s.at[3])
                for w in range(NG)]

    def src_group(g):
        return min(g, NG - 1) if isinstance(g, int) else jnp.minimum(g, NG - 1)

    def cp_conv(g):
        src = src_group(g)
        return [pltpu.make_async_copy(fk_hbm.at[col(src), :], fk_v.at[g], sem_g.at[g])] + [
            pltpu.make_async_copy(a.at[:, col(src)], dst.at[g], sem_g.at[g])
            for a, dst in ((ak_hbm, ak_v), (av_hbm, av_v), (aq_hbm, aq_v))]

    def cp_wk(g):
        return [pltpu.make_async_copy(wk_hbm.at[:, col(g)], wk_v.at[g], sem_s.at[4 + g])]

    def cp_wqv(g):
        return [pltpu.make_async_copy(src.at[:, col(g)], dst.at[g], sem_s.at[4 + NG + g])
                for src, dst in ((wq_hbm, wq_v), (wv_hbm, wv_v))]

    def cp_w(windows):
        return [c for g in windows for c in cp_wk(g) + cp_wqv(g)]

    def cp_ya(g):
        return pltpu.make_async_copy(ya_s.at[g], out_hbm.at[:, col(g)], sem_out.at[g])

    def cp_yb(s, part):
        lo, n = ((0, L - T), (L - T, T))[part]
        r0 = s * L + lo if isinstance(s, int) else pl.multiple_of(s * L + lo, T)
        return pltpu.make_async_copy(yb_s.at[s, pl.ds(lo, n)], out_hbm.at[pl.ds(r0, n), D:2 * D],
                                     sem_out.at[NG + 2 * s + part])

    PRE = cfg["npre"]
    _start(cp_x(0) + cp_w((0,)))
    _start(cp_x(1) + cp_conv(0), priority=1)

    for i in range(8):
        zero_s[i] = 0
    r_i = lax.broadcasted_iota(I32, (T, T), 0)
    c_i = lax.broadcasted_iota(I32, (T, T), 1)
    mask_s[...] = jnp.where(r_i <= c_i, 0.0, NEG)

    def x_tile(t):
        return jnp.concatenate([_ld(x_v, (c,), T * t, T) for c in range(NG)], axis=1)

    def transpose_w(g):
        for c in range(NG):
            wt_s[g, c, 0:T, :] = _ld(wq_v, (g,), T * c, T).T
            wt_s[g, c, T:2 * T, :] = _ld(wv_v, (g,), T * c, T).T

    def proj_k(g, t, z):
        rows = slice(T * t, T * (t + 1))
        k = _nn(x_tile(t), _ld(wk_v, (g,), 0, D))
        k_s[g, rows, :] = k.astype(BF)
        pk_s[g, rows, :] = _phi(k).astype(BF)

    def straddle(g, t, z):
        words = slice(T * t // 2, T * (t + 1) // 2)
        gp = g - 1 if isinstance(g, int) else jnp.maximum(g - 1, 0)
        ku = k_s.bitcast(U32)
        ku[NG + g, words, :] = jnp.where(c_i[:T // 2] < 64, ku[g + z, words, :], ku[gp + z, words, :])

    def proj_qv(g, t, z):
        wt = jnp.concatenate([_ld(wt_s, (g + z, c), 0, 2 * T) for c in range(NG)], axis=1)
        qv = _nt(wt, x_tile(t))
        q = qv[:T]
        q_s[t, col(g), :] = (q * QSCALE).astype(BF)
        pq_s[t, col(g), :] = _phi(q).astype(BF)
        v_s[t, col(g), :] = qv[T:]

    def project(windows, z):
        jobs = [(g, t) for g in windows for t in range(PRE)]
        for g in windows:
            transpose_w(g)
        for fn in (proj_k, proj_qv):
            for g, t in jobs:
                fn(g, t, z)
        for g, t in jobs:
            if g:
                straddle(g, t, z)

    with _scope("ph_wait0"):
        _wait(cp_x(0) + cp_w((0,)))
    with _scope("ph_10"):
        z0 = zero_s[0]
        num_s[0] = jnp.zeros((NQ, D, T), F32)
        rden_s[0:NQ] = jnp.zeros((NQ, H, T), F32)
        _start(cp_w((1,)) + cp_small())
        project((0,), z0)
        _start(cp_w((2, 3, 4)))
        _wait(cp_w((1,)) + cp_small())
        taps = sk_v[...].astype(F32)
        dvec = dd_v[...].astype(F32).reshape(1, D)
        for g in range(NG):
            for j in range(4):
                par_s[g, j] = jnp.broadcast_to(taps[j:j + 1, T * g:T * (g + 1)], (8, T))
            par_s[g, 4] = jnp.broadcast_to(dvec[:, T * g:T * (g + 1)], (8, T))
        gate = jax.nn.sigmoid(beta_v[...].astype(F32).reshape(1, H)).astype(BF).astype(F32)
        hr = lax.broadcasted_iota(I32, (H, H), 0)
        hc = lax.broadcasted_iota(I32, (H, H), 1)
        gcol = jnp.sum(jnp.where(hr == hc, jnp.broadcast_to(gate, (H, H)), 0.0), axis=1, keepdims=True)
        g_s[...] = jnp.broadcast_to(gcol, (H, T))
        project((1,), z0)
        _wait(cp_w((2, 3, 4)))
        project((2, 3, 4), z0)
        _wait(cp_x(1) + cp_conv(0))
        _start(cp_conv(1))
        _start(cp_wo(), priority=1)

    def phase1(g, carry):
        zeros = [zero_s[i] for i in range(5)]
        fwd = lambda: _ld(dft_v, (), 0, 2 * T)

        def filt(j):
            kf_s[j] = _nt(fwd(), fk_v[g, :, T * j:T * (j + 1)])

        def kv(a):
            cur = _ld(ak_v, (g,), T * a, T).astype(F32)
            if a == 0:
                prev = jnp.zeros((8, T), F32)
            else:
                prev = _ld(ak_v, (g,), T * a - 16, 16).astype(F32)[8:]
            ext = jnp.concatenate([prev, cur], axis=0)
            acc = cur * par_s[g, 0][0:1]
            for j in range(1, 4):
                acc = acc + ext[8 - j:8 - j + T] * par_s[g, j][0:1]
            u = (acc * _ld(av_v, (g,), T * a, T).astype(F32)).astype(BF)
            kv_s[T * a:T * (a + 1), :] = u
            uf_s[a] = _nn(fwd(), u)

        def slab(s):
            re, im = slice(16 * s, 16 * s + 8), slice(16 * s + 8, 16 * s + 16)
            t1_s, t2_s = t_ring[2 * (s % cfg['tr'])], t_ring[2 * (s % cfg['tr']) + 1]
            for part, dst, z in ((re, t1_s, zeros[0]), (im, t2_s, zeros[1])):
                t = _short_conv([uf_s[a + z, part, :] for a in range(NB)],
                                [kf_s[j + z, part, :] for j in range(NB)])
                for c in range(NB):
                    dst[0, c] = t[c]
            z = zeros[2]
            t = _short_conv([uf_s[a + z, re, :] + uf_s[a + z, im, :] for a in range(NB)],
                            [kf_s[j + z, re, :] + kf_s[j + z, im, :] for j in range(NB)])
            pr = pi = None
            for c in range(NB):
                rr, ii = t1_s[z, c], t2_s[z, c]
                wr, wi = rr - ii, t[c] - rr - ii
                zr, zi = (wr, wi) if c == 0 else (wr + pi, wi - pr)
                pr, pi = wr, wi
                z_s[c, 16 * s:16 * s + 16, :] = jnp.concatenate([zr, zi], axis=0).astype(BF)

        def inv(c):
            z = zeros[3]
            y = (_nn(_ld(dft_v, (), 2 * T, T), _ld(z_s, (c + z,), 0, T))
                 + _nn(_ld(dft_v, (), 3 * T, T), _ld(z_s, (c + z,), T, T)))
            y = y + _ld(kv_s, (), T * c + z, T).astype(F32) * par_s[g, 4][0:1]
            ya_s[g, T * c:T * (c + 1), :] = (_ld(aq_v, (g,), T * c, T).astype(F32) * y).astype(BF)

        lead = cfg["lead"]
        for j in range(NB + lead):
            if j < NB:
                filt(j)
            if j >= lead:
                kv(j - lead)
        for t in range(cfg["npre"], NB):
            proj_k(g, t, zeros[4])
            proj_qv(g, t, zeros[4])
            if t - cfg["xlag"] >= cfg["npre"]:
                straddle(g, t - cfg["xlag"], zeros[4])
        for t in range(NB - cfg["xlag"], NB):
            straddle(g, t, zeros[4])
        for s in range(NB):
            slab(s)
        for c in range(NB):
            inv(c)
        _start(cp_conv(g + 2))
        _wait(cp_conv(g + 1))
        return carry

    with _scope("ph_1"):
        lax.fori_loop(0, NG, phase1, 0)

    gcolv = g_s[...]
    mem = [None] * NG
    scope = _scope('ph_mem')
    scope.__enter__()
    for s in range(NSEG - 1):
        lhs = []
        for w in range(NG):
            n = _R1[w] - _R0[w]
            vv = jnp.concatenate([v_s[NQ * s + i, _R0[w]:_R1[w], :] for i in range(NQ)], axis=1)
            vv = jnp.concatenate([vv, jnp.ones((8, L), F32)], axis=0)
            upd = _nn(vv, _ld(pk_s, (w,), L * s, L))
            mem[w] = upd if mem[w] is None else mem[w] + upd
            rh = _head_of(lax.broadcasted_iota(I32, (n, T), 0) + _R0[w])
            ch = _head_of(lax.broadcasted_iota(I32, (n, T), 1) + T * w)
            zh = lax.broadcasted_iota(I32, (8, T), 0) + _H0[w]
            ch8 = _head_of(lax.broadcasted_iota(I32, (8, T), 1) + T * w)
            lhs.append(jnp.concatenate([jnp.where(rh == ch, mem[w][:n], 0.0),
                                        jnp.where(zh == ch8, mem[w][n:], 0.0)], axis=0))
        for i in range(NQ):
            t = NQ * (s + 1) + i
            res = [_nn(lhs[w], _ld(pq_s, (t,), T * w, T)) for w in range(NG)]
            den = None
            for w in range(NG):
                lo = _R0[w] if w == 0 else _R1[w - 1]
                hi = _R1[w] if w == NG - 1 else _R0[w + 1]
                num_s[s + 1, i, lo:hi, :] = res[w][lo - _R0[w]:hi - _R0[w]]
                if w + 1 < NG:
                    num_s[s + 1, i, hi:_R1[w], :] = (res[w][hi - _R0[w]:_R1[w] - _R0[w]]
                                                     + res[w + 1][:_R1[w] - hi])
                part = jnp.concatenate(
                    ([jnp.zeros((_H0[w], T), F32)] if _H0[w] else [])
                    + [res[w][_R1[w] - _R0[w]:], jnp.zeros((H - _H0[w], T), F32)], axis=0)[:H]
                den = part if den is None else den + part
            rden_s[t] = gcolv / (den + 1e-6)

    scope.__exit__(None, None, None)
    _wait(cp_wo())
    _start([cp_ya(g) for g in range(NG)])

    tiles = [(i, h, j) for i in cfg["iorder"] for h in range(H) for j in range(i + 1)]

    def segment(s, carry):
        zeros = [zero_s[5 + i] for i in range(2)]
        sub8 = lax.broadcasted_iota(I32, (8, T), 0)
        t0 = pl.multiple_of(s * L, L)
        qws, mx, pvals, acc, fin, held = {}, {}, {}, {}, {}, {}

        def q_weights(i, h):
            f0 = DH * h
            blocks = [jnp.zeros((8, T), U32)] * 8
            for b in (f0 // 16, f0 // 16 + 1):
                blk = q_s.bitcast(U32)[NQ * s + i, 8 * b:8 * b + 8, :]
                lo, hi = f0 // 2 - 8 * b, (f0 + DH) // 2 - 8 * b
                if lo > 0:
                    blk = jnp.where(sub8 >= lo, blk, jnp.uint32(0))
                if hi < 8:
                    blk = jnp.where(sub8 < hi, blk, jnp.uint32(0))
                blocks[b % 8] = blk
            return pltpu.bitcast(jnp.concatenate(blocks, axis=0), BF)

        def q_shared(i, m):
            f0 = 2 * DH * m
            low = lax.broadcasted_iota(I32, (8, T), 1) < 64
            blocks = [jnp.zeros((8, T), U32)] * 8
            for b in range(f0 // 16, (f0 + 2 * DH - 1) // 16 + 1):
                blk = q_s.bitcast(U32)[NQ * s + i, 8 * b:8 * b + 8, :]
                row = sub8 + 8 * b - f0 // 2
                in_a = (row >= 0) & (row < DH // 2) & low
                in_b = (row >= DH // 2) & (row < DH) & jnp.logical_not(low)
                blocks[b % 8] = jnp.where(in_a, pltpu.roll(blk, 64, 1), jnp.where(in_b, blk, jnp.uint32(0)))
            return pltpu.bitcast(jnp.concatenate(blocks, axis=0), BF)

        def keep(n, r0, sc):
            i, h, _ = tiles[n]
            m8 = jnp.max(sc.reshape(sc.shape[0] // 8, 8, T), axis=0)
            mx[i, h] = m8 if (i, h) not in mx else jnp.maximum(mx[i, h], m8)
            s_ring[n % RING][0, r0:r0 + sc.shape[0], :] = sc

        def stage_a(n):
            i, h, j = tiles[n]
            f0 = 2 * DH * (h // 2)
            wb, wa = f0 // T, (f0 + 2 * DH - 1) // T
            win = (wb if wa == wb else NG + wa,)
            if (i, h) not in qws:
                qws[i, h] = q_weights(i, h)
            merge = cfg["merge"] and i > 0
            if merge and j == i - 1:
                sc = _nn(_ld(k_s, win, t0 + T * j, T + 64), qws[i, h])
                keep(n, 0, sc[:T])
                keep(n + 1, 0, sc[T:] + mask_s[0:64, :])
            elif j < i:
                keep(n, 0, _nn(_ld(k_s, win, t0 + T * j, T), qws[i, h]))
            else:
                if not merge:
                    keep(n, 0, _nn(_ld(k_s, win, t0 + T * j, 64), qws[i, h]) + mask_s[0:64, :])
                if h % 2 == 0:
                    sh = _nn(_ld(k_s, win, t0 + T * j + 64, 64), q_shared(i, h // 2))
                    keep(n, 64, pltpu.roll(sh, 64, 1) + mask_s[64:T, :])
                    keep(n + i + 1, 64, sh + mask_s[64:T, :])

        def stage_b(n):
            i, h, j = tiles[n]
            if (i, h) not in fin:
                fin[i, h] = jnp.max(mx.pop((i, h)), axis=0, keepdims=True)
            pvals[n] = jnp.exp2(s_ring[n % RING][zeros[0]] - fin[i, h]).astype(BF)

        def stage_c(n):
            i, h, j = tiles[n]
            base = (h // 2) * 2 * DH + (h % 2) * 16
            vv = v_s[NQ * s + j, base:base + 24, :]
            if h % 2 == 0:
                vv = jnp.concatenate([vv[:16], jnp.where(sub8 < 4, vv[16:], 1.0)], axis=0)
            else:
                vv = jnp.concatenate([jnp.where(sub8 >= 4, vv[:8], 1.0), vv[8:]], axis=0)
            o = _nn(vv, pvals.pop(n))
            acc[i, h] = o if j == 0 else acc[i, h] + o
            if j == i:
                a = acc.pop((i, h))
                den = a[DH:DH + 1] if h % 2 == 0 else a[0:1]
                w_dot = (1.0 - g_s[h:h + 1, :]) / den
                w_mem = rden_s[NQ * s + i, h:h + 1, :]
                o = a * w_dot + num_s[s, i, base:base + 24, :] * w_mem
                if h % 2 == 0:
                    ot_s[i][0, base:base + 16, :] = o[:16]
                    held[i] = o[16:]
                else:
                    mid = jnp.where(sub8 < 4, held.pop(i), o[:8])
                    ot_s[i][0, base:base + 24, :] = jnp.concatenate([mid, o[8:]], axis=0)

        def out_proj(i):
            ot = jnp.concatenate([ot_s[i][zeros[1], T * w:T * (w + 1), :].T for w in range(NG)], axis=1)
            wo = jnp.concatenate([_ld(wo_v, (c,), 0, D) for c in range(NG)], axis=1)
            yb_s[s, T * i:T * (i + 1), :] = _nn(ot.astype(BF), wo).astype(BF)

        n = len(tiles)
        lb, lc, grp = cfg["lagB"], cfg["lagC"], cfg["G"]
        last = {i: max(k for k in range(n) if tiles[k][0] == i) for i in cfg["iorder"]}
        todo = list(cfg["iorder"])
        for tt in range(0, n + lb + lc, grp):
            for k in range(tt, tt + grp):
                if k < n:
                    stage_a(k)
            for k in range(tt, tt + grp):
                if 0 <= k - lb < n:
                    stage_b(k - lb)
            for k in range(tt, tt + grp):
                if 0 <= k - lb - lc < n:
                    stage_c(k - lb - lc)
            if len(todo) > 3 and tt - lb - lc > last[todo[0]] + cfg["olag"]:
                out_proj(todo.pop(0))
            if len(todo) == 3 and tt + grp >= n:
                out_proj(todo.pop(0))
        for i in todo:
            if i == NQ - 1:
                cp_yb(s, 0).start()
            out_proj(i)
        cp_yb(s, 1).start()
        return carry

    with _scope("ph_2"):
        lax.fori_loop(0, cfg['n'], lambda q, c: segment(q & 3, c), 0)

    with _scope("ph_tail"):
        _wait(cp_conv(NG + 1))
        for g in range(NG):
            cp_ya(g).wait()
        for s in range(cfg['n']):
            cp_yb(s & 3, 0).wait()
            cp_yb(s & 3, 1).wait()


@jax.jit
def pallas_concat_heads__ssm_conv_h3__memory_aug_infini_attn__prompt_kernel(
    A_q, A_k, A_v, A_shift_k, A_ssm_k, A_ssm_D, B_x, B_wq, B_wk, B_wv, B_wo, B_beta,
):
    hbm = pl.BlockSpec(memory_space=pl.ANY)
    scratch = CFG['perm'](_scratch())

    def body(*refs):
        _kernel(*refs[:14], **dict(zip(scratch, refs[14:])))

    out = pl.pallas_call(
        body,
        out_shape=jax.ShapeDtypeStruct((S, 2 * D), BF),
        in_specs=[hbm] * 13,
        out_specs=hbm,
        scratch_shapes=list(scratch.values()),
        compiler_params=pltpu.CompilerParams(vmem_limit_bytes=100 * 1024 * 1024),
        name="h3_infini",
    )(A_q.reshape(S, D), A_k.reshape(S, D), A_v.reshape(S, D), A_shift_k.T, A_ssm_k, A_ssm_D,
      B_x.reshape(S, D), B_wq, B_wk, B_wv, B_wo, B_beta, _DFT)
    return out.reshape(1, S, 2 * D)
```

```python
import jax
import jax.numpy as jnp
import numpy as np
from jax import lax
import jax.experimental.pallas as pl
import jax.experimental.pallas.tpu as pltpu

BF = jnp.bfloat16
F32 = jnp.float32
U32 = jnp.uint32
I32 = jnp.int32

S = 2048
D = 640
H = 32
DH = 20
NSEG = 4
L = S // NSEG
T = 128
NB = S // T
NQ = L // T
NG = D // T
LOG2E = 1.4426950408889634
QSCALE = DH ** -0.5 * LOG2E
NEG = -1e9 * LOG2E

PRE = 5
NSET = 4
RING = 32
LAG_EXP = 12
LAG_PV = 4
STEP = 4
Q_GROUPS = ((2, 1), (3, 0))
OUT_ORDER = (2, 1, 0, 3)


def _dft_matrices():
    theta = (0.5 * np.pi + 2.0 * np.pi * np.arange(T)) / T
    ang = theta[:, None] * np.arange(T)[None, :]
    f = np.stack([np.cos(ang).reshape(NB, 8, T), np.sin(ang).reshape(NB, 8, T)], axis=1)
    f = f.reshape(2 * T, T)
    g = (f.T / T).reshape(T, 2, T).transpose(1, 0, 2).reshape(2 * T, T)
    return np.concatenate([f, g], axis=0).astype(BF)


_DFT = _dft_matrices()

_H0 = [(T * w) // DH for w in range(NG)]
_H1 = [(T * w + T - 1) // DH for w in range(NG)]
_R0 = [(DH * h) // 8 * 8 for h in _H0]
_R1 = [-(-(DH * (h + 1)) // 8) * 8 for h in _H1]


def _phi(t):
    return jnp.where(t > 0, t + 1.0, jnp.exp(t))


def _head_of(idx):
    return (idx * 3277) >> 16


def _ld(ref, idx, r0, n):
    if isinstance(r0, int):
        rows = pl.ds(r0 // 2, n // 2)
    else:
        rows = pl.ds(pl.multiple_of(r0 // 2, 8), n // 2)
    return pltpu.bitcast(ref.bitcast(U32)[(*idx, rows, slice(None))], BF)


def _nn(a, b):
    return lax.dot_general(a, b, (((1,), (0,)), ((), ())), preferred_element_type=F32)


def _nt(a, b):
    return lax.dot_general(a, b, (((1,), (1,)), ((), ())), preferred_element_type=F32)


def _short_conv(us, ks):
    out = []
    for c in range(NB):
        acc = us[c] * ks[0]
        for j in range(1, c + 1):
            acc = acc + us[c - j] * ks[j]
        out.append(acc)
    return out


def _start(copies, priority=0):
    for c in copies:
        c.start(priority=priority)


def _wait(copies):
    for c in copies:
        c.wait()


def _scratch():
    vm = pltpu.VMEM
    return dict(
        wo_v=vm((NG, D, T), BF),
        k_s=vm((2 * NG, S, T), BF),
        q_s=vm((NB, D, T), BF),
        v_s=vm((NB, D, T), F32),
        num_s=vm((NSEG, NQ, D, T), F32),
        rden_s=vm((NB, H, T), F32),
        yb_s=vm((NSEG, L, D), BF),
        mask_s=vm((T, T), F32),
        g_s=vm((H, T), F32),
        **{f"ot{i}": vm((1, D, T), F32) for i in range(NQ)},
        **{f"sr{i}": vm((1, T, T), F32) for i in range(RING)},
        aq_v=vm((NG + 2, S, T), BF),
        ak_v=vm((NG + 2, S, T), BF),
        av_v=vm((NG + 2, S, T), BF),
        fk_v=vm((NG + 2, T, S), BF),
        x_v=vm((NG, S, T), BF),
        wq_v=vm((NG, D, T), BF),
        wk_v=vm((NG, D, T), BF),
        wv_v=vm((NG, D, T), BF),
        dft_v=vm((4 * T, T), BF),
        wt_s=vm((NG, NG, 2 * T, T), BF),
        kv_s=vm((S, T), BF),
        uf_s=vm((NB, 2 * T, T), F32),
        kf_s=vm((NB, 2 * T, T), F32),
        z_s=vm((NB, 2 * T, T), BF),
        ya_s=vm((NG, S, T), BF),
        pk_s=vm((NG, S, T), BF),
        pq_s=vm((NB, D, T), BF),
        par_s=vm((NG, 5, 8, T), F32),
        **{f"tr{i}": vm((1, NB, 8, T), F32) for i in range(2 * NSET)},
        sk_v=vm((4, D), BF),
        dd_v=vm((D,), BF),
        beta_v=vm((H,), BF),
        zero_s=pltpu.SMEM((8,), I32),
        sem_s=pltpu.SemaphoreType.DMA((2 + 2 * NG,)),
        sem_g=pltpu.SemaphoreType.DMA((NG + 2,)),
        sem_x=pltpu.SemaphoreType.DMA((2,)),
        sem_out=pltpu.SemaphoreType.DMA((NG + 2 * NSEG,)),
    )


def _kernel(aq_hbm, ak_hbm, av_hbm, sk_hbm, fk_hbm, dd_hbm, x_hbm, wq_hbm, wk_hbm, wv_hbm,
            wo_hbm, beta_hbm, dft_hbm, out_hbm, *, aq_v, ak_v, av_v, fk_v, x_v, wq_v, wk_v, wv_v,
            wo_v, sk_v, dd_v, beta_v, dft_v, wt_s, kv_s, uf_s, kf_s, z_s, ya_s, k_s, q_s, v_s,
            pk_s, pq_s, num_s, rden_s, yb_s, mask_s, par_s, g_s, zero_s, sem_s, sem_g, sem_x,
            sem_out, **rings):
    ot_s = [rings[f"ot{i}"] for i in range(NQ)]
    s_ring = [rings[f"sr{i}"] for i in range(RING)]
    t_ring = [rings[f"tr{i}"] for i in range(2 * NSET)]

    def col(g):
        return pl.ds(g * T if isinstance(g, int) else pl.multiple_of(g * T, T), T)

    def cp_small():
        return [pltpu.make_async_copy(src, dst, sem_s.at[0]) for src, dst in
                ((sk_hbm, sk_v), (dd_hbm, dd_v), (beta_hbm, beta_v), (dft_hbm, dft_v))]

    def cp_wo():
        return [pltpu.make_async_copy(wo_hbm.at[:, col(w)], wo_v.at[w], sem_s.at[1])
                for w in range(NG)]

    def cp_w(windows):
        cs = []
        for g in windows:
            cs.append(pltpu.make_async_copy(wk_hbm.at[:, col(g)], wk_v.at[g], sem_s.at[2 + g]))
            cs += [pltpu.make_async_copy(src.at[:, col(g)], dst.at[g], sem_s.at[2 + NG + g])
                   for src, dst in ((wq_hbm, wq_v), (wv_hbm, wv_v))]
        return cs

    def cp_x(part):
        lo, hi = ((0, PRE), (PRE, NB))[part]
        rows = pl.ds(T * lo, T * (hi - lo))
        return [pltpu.make_async_copy(x_hbm.at[rows, col(w)], x_v.at[w, rows], sem_x.at[part])
                for w in range(NG)]

    def cp_conv(g):
        src = min(g, NG - 1) if isinstance(g, int) else jnp.minimum(g, NG - 1)
        return [pltpu.make_async_copy(fk_hbm.at[col(src), :], fk_v.at[g], sem_g.at[g])] + [
            pltpu.make_async_copy(a.at[:, col(src)], dst.at[g], sem_g.at[g])
            for a, dst in ((ak_hbm, ak_v), (av_hbm, av_v), (aq_hbm, aq_v))]

    def cp_ya(g):
        return pltpu.make_async_copy(ya_s.at[g], out_hbm.at[:, col(g)], sem_out.at[g])

    def cp_yb(s, part):
        lo, n = ((0, L - T), (L - T, T))[part]
        r0 = s * L + lo if isinstance(s, int) else pl.multiple_of(s * L + lo, T)
        return pltpu.make_async_copy(yb_s.at[s, pl.ds(lo, n)], out_hbm.at[pl.ds(r0, n), D:2 * D],
                                     sem_out.at[NG + 2 * s + part])

    _start(cp_x(0) + cp_w((0,)))
    _start(cp_x(1) + cp_conv(0), priority=1)

    for i in range(8):
        zero_s[i] = 0
    r_i = lax.broadcasted_iota(I32, (T, T), 0)
    c_i = lax.broadcasted_iota(I32, (T, T), 1)
    mask_s[...] = jnp.where(r_i <= c_i, 0.0, NEG)

    def x_tile(t):
        return jnp.concatenate([_ld(x_v, (c,), T * t, T) for c in range(NG)], axis=1)

    def proj_k(g, t, z):
        rows = slice(T * t, T * (t + 1))
        k = _nn(x_tile(t), _ld(wk_v, (g,), 0, D))
        k_s[g, rows, :] = k.astype(BF)
        if t < NB - NQ:
            pk_s[g, rows, :] = _phi(k).astype(BF)

    def straddle(g, t, z):
        words = slice(T * t // 2, T * (t + 1) // 2)
        gp = g - 1 if isinstance(g, int) else jnp.maximum(g - 1, 0)
        ku = k_s.bitcast(U32)
        ku[NG + g, words, :] = jnp.where(c_i[:T // 2] < 64, ku[g + z, words, :], ku[gp + z, words, :])

    def proj_qv(g, t, z):
        wt = jnp.concatenate([_ld(wt_s, (g + z, c), 0, 2 * T) for c in range(NG)], axis=1)
        qv = _nt(wt, x_tile(t))
        q = qv[:T]
        q_s[t, col(g), :] = (q * QSCALE).astype(BF)
        if t >= NQ:
            pq_s[t, col(g), :] = _phi(q).astype(BF)
        v_s[t, col(g), :] = qv[T:]

    def project_first(windows, z):
        for g in windows:
            for c in range(NG):
                wt_s[g, c, 0:T, :] = _ld(wq_v, (g,), T * c, T).T
                wt_s[g, c, T:2 * T, :] = _ld(wv_v, (g,), T * c, T).T
        jobs = [(g, t) for g in windows for t in range(PRE)]
        for fn in (proj_k, proj_qv):
            for g, t in jobs:
                fn(g, t, z)
        for g, t in jobs:
            if g:
                straddle(g, t, z)

    _wait(cp_x(0) + cp_w((0,)))
    z0 = zero_s[0]
    num_s[0] = jnp.zeros((NQ, D, T), F32)
    rden_s[0:NQ] = jnp.zeros((NQ, H, T), F32)
    _start(cp_w((1,)) + cp_small())
    project_first((0,), z0)
    _start(cp_w((2, 3, 4)))
    _wait(cp_w((1,)) + cp_small())
    taps = sk_v[...].astype(F32)
    dvec = dd_v[...].astype(F32).reshape(1, D)
    for g in range(NG):
        for j in range(4):
            par_s[g, j] = jnp.broadcast_to(taps[j:j + 1, T * g:T * (g + 1)], (8, T))
        par_s[g, 4] = jnp.broadcast_to(dvec[:, T * g:T * (g + 1)], (8, T))
    gate = jax.nn.sigmoid(beta_v[...].astype(F32).reshape(1, H)).astype(BF).astype(F32)
    hr = lax.broadcasted_iota(I32, (H, H), 0)
    hc = lax.broadcasted_iota(I32, (H, H), 1)
    gcol = jnp.sum(jnp.where(hr == hc, jnp.broadcast_to(gate, (H, H)), 0.0), axis=1, keepdims=True)
    g_s[...] = jnp.broadcast_to(gcol, (H, T))
    project_first((1,), z0)
    _wait(cp_w((2, 3, 4)))
    project_first((2, 3, 4), z0)
    _wait(cp_x(1) + cp_conv(0))
    _start(cp_conv(1))
    _start(cp_wo(), priority=1)

    def group(g, carry):
        zeros = [zero_s[i] for i in range(5)]

        def filt(j):
            kf_s[j] = _nt(_ld(dft_v, (), 0, 2 * T), fk_v[g, :, T * j:T * (j + 1)])

        def kv(a):
            cur = _ld(ak_v, (g,), T * a, T).astype(F32)
            if a == 0:
                prev = jnp.zeros((8, T), F32)
            else:
                prev = _ld(ak_v, (g,), T * a - 16, 16).astype(F32)[8:]
            ext = jnp.concatenate([prev, cur], axis=0)
            acc = cur * par_s[g, 0][0:1]
            for j in range(1, 4):
                acc = acc + ext[8 - j:8 - j + T] * par_s[g, j][0:1]
            u = (acc * _ld(av_v, (g,), T * a, T).astype(F32)).astype(BF)
            kv_s[T * a:T * (a + 1), :] = u
            uf_s[a] = _nn(_ld(dft_v, (), 0, 2 * T), u)

        def slab(s):
            re, im = slice(16 * s, 16 * s + 8), slice(16 * s + 8, 16 * s + 16)
            rr_s, ii_s = t_ring[2 * (s % NSET)], t_ring[2 * (s % NSET) + 1]
            for part, dst, z in ((re, rr_s, zeros[0]), (im, ii_s, zeros[1])):
                t = _short_conv([uf_s[a + z, part, :] for a in range(NB)],
                                [kf_s[j + z, part, :] for j in range(NB)])
                for c in range(NB):
                    dst[0, c] = t[c]
            z = zeros[2]
            t = _short_conv([uf_s[a + z, re, :] + uf_s[a + z, im, :] for a in range(NB)],
                            [kf_s[j + z, re, :] + kf_s[j + z, im, :] for j in range(NB)])
            pr = pi = None
            for c in range(NB):
                rr, ii = rr_s[z, c], ii_s[z, c]
                wr, wi = rr - ii, t[c] - rr - ii
                zr, zi = (wr, wi) if c == 0 else (wr + pi, wi - pr)
                pr, pi = wr, wi
                z_s[c, 16 * s:16 * s + 16, :] = jnp.concatenate([zr, zi], axis=0).astype(BF)

        def inv(c):
            z = zeros[3]
            y = (_nn(_ld(dft_v, (), 2 * T, T), _ld(z_s, (c + z,), 0, T))
                 + _nn(_ld(dft_v, (), 3 * T, T), _ld(z_s, (c + z,), T, T)))
            y = y + _ld(kv_s, (), T * c + z, T).astype(F32) * par_s[g, 4][0:1]
            ya_s[g, T * c:T * (c + 1), :] = (_ld(aq_v, (g,), T * c, T).astype(F32) * y).astype(BF)

        for j in range(NB + 1):
            if j < NB:
                filt(j)
            if j:
                kv(j - 1)
        for t in range(PRE, NB):
            proj_k(g, t, zeros[4])
            proj_qv(g, t, zeros[4])
            if t > PRE:
                straddle(g, t - 1, zeros[4])
        straddle(g, NB - 1, zeros[4])
        for s in range(NB):
            slab(s)
        for c in range(NB):
            inv(c)
        _start(cp_conv(g + 2))
        _wait(cp_conv(g + 1))
        return carry

    lax.fori_loop(0, NG, group, 0)

    gcolv = g_s[...]
    mem = [None] * NG
    for s in range(NSEG - 1):
        lhs = []
        for w in range(NG):
            n = _R1[w] - _R0[w]
            vv = jnp.concatenate([v_s[NQ * s + i, _R0[w]:_R1[w], :] for i in range(NQ)], axis=1)
            vv = jnp.concatenate([vv, jnp.ones((8, L), F32)], axis=0)
            upd = _nn(vv, _ld(pk_s, (w,), L * s, L))
            mem[w] = upd if mem[w] is None else mem[w] + upd
            rh = _head_of(lax.broadcasted_iota(I32, (n, T), 0) + _R0[w])
            ch = _head_of(lax.broadcasted_iota(I32, (n, T), 1) + T * w)
            zh = lax.broadcasted_iota(I32, (8, T), 0) + _H0[w]
            ch8 = _head_of(lax.broadcasted_iota(I32, (8, T), 1) + T * w)
            lhs.append(jnp.concatenate([jnp.where(rh == ch, mem[w][:n], 0.0),
                                        jnp.where(zh == ch8, mem[w][n:], 0.0)], axis=0))
        for i in range(NQ):
            t = NQ * (s + 1) + i
            res = [_nn(lhs[w], _ld(pq_s, (t,), T * w, T)) for w in range(NG)]
            den = None
            for w in range(NG):
                lo = _R0[w] if w == 0 else _R1[w - 1]
                hi = _R1[w] if w == NG - 1 else _R0[w + 1]
                num_s[s + 1, i, lo:hi, :] = res[w][lo - _R0[w]:hi - _R0[w]]
                if w + 1 < NG:
                    num_s[s + 1, i, hi:_R1[w], :] = (res[w][hi - _R0[w]:_R1[w] - _R0[w]]
                                                     + res[w + 1][:_R1[w] - hi])
                part = jnp.concatenate(
                    ([jnp.zeros((_H0[w], T), F32)] if _H0[w] else [])
                    + [res[w][_R1[w] - _R0[w]:], jnp.zeros((H - _H0[w], T), F32)], axis=0)[:H]
                den = part if den is None else den + part
            rden_s[t] = gcolv / (den + 1e-6)

    _wait(cp_wo())
    _start([cp_ya(g) for g in range(NG)])

    tiles = [(i, h, j) for grp in Q_GROUPS for m in range(H // 2) for i in grp
             for h in (2 * m, 2 * m + 1) for j in range(i + 1)]

    def segment(s, carry):
        zeros = [zero_s[5 + i] for i in range(2)]
        sub8 = lax.broadcasted_iota(I32, (8, T), 0)
        lane8 = lax.broadcasted_iota(I32, (8, T), 1)
        t0 = pl.multiple_of(s * L, L)
        qws, mx, pvals, acc, fin, held, ksp = {}, {}, {}, {}, {}, {}, {}

        def q_blocks(i, h):
            f0 = DH * h
            for b in (f0 // 16, f0 // 16 + 1):
                blk = q_s.bitcast(U32)[NQ * s + i, 8 * b:8 * b + 8, :]
                lo, hi = f0 // 2 - 8 * b, (f0 + DH) // 2 - 8 * b
                if lo > 0:
                    blk = jnp.where(sub8 >= lo, blk, jnp.uint32(0))
                if hi < 8:
                    blk = jnp.where(sub8 < hi, blk, jnp.uint32(0))
                yield b, blk

        def q_weights(i, h):
            blocks = [jnp.zeros((8, T), U32)] * 8
            for b, blk in q_blocks(i, h):
                blocks[b % 8] = blk
            return pltpu.bitcast(jnp.concatenate(blocks, axis=0), BF)

        def q_shared(i, m):
            f0 = 2 * DH * m
            blocks = [jnp.zeros((8, T), U32)] * 8
            for b in range(f0 // 16, (f0 + 2 * DH - 1) // 16 + 1):
                blk = q_s.bitcast(U32)[NQ * s + i, 8 * b:8 * b + 8, :]
                row = sub8 + 8 * b - f0 // 2
                in_a = (row >= 0) & (row < DH // 2) & (lane8 < 64)
                in_b = (row >= DH // 2) & (row < DH) & (lane8 >= 64)
                blocks[b % 8] = jnp.where(in_a, pltpu.roll(blk, 64, 1),
                                          jnp.where(in_b, blk, jnp.uint32(0)))
            return pltpu.bitcast(jnp.concatenate(blocks, axis=0), BF)

        def q_split(i, h):
            blocks = [jnp.zeros((8, T), U32)] * 8
            for b, blk in q_blocks(i, h):
                blocks[b % 8] = jnp.where(lane8 >= 32, blk, jnp.uint32(0))
                blocks[(b + 4) % 8] = jnp.where(lane8 < 32, pltpu.roll(blk, 32, 1), jnp.uint32(0))
            return pltpu.bitcast(jnp.concatenate(blocks, axis=0), BF)

        def k_split(win, i, m):
            ku = k_s.bitcast(U32)
            r0 = pl.multiple_of((t0 + T * i) // 2, 8)
            first = ku[win, pl.ds(r0 + 16, 16), :]
            second = pltpu.roll(ku[win, pl.ds(r0 + 48, 16), :], 64, 1)
            lane = lax.broadcasted_iota(I32, (16, T), 1)
            return pltpu.bitcast(jnp.where(((lane - 2 * DH * m) & (T - 1)) < 64, first, second), BF)

        def keep(n, r0, sc):
            i, h, _ = tiles[n]
            m8 = jnp.max(sc.reshape(sc.shape[0] // 8, 8, T), axis=0)
            mx[i, h] = m8 if (i, h) not in mx else jnp.maximum(mx[i, h], m8)
            s_ring[n % RING][0, r0:r0 + sc.shape[0], :] = sc

        def logits(n):
            i, h, j = tiles[n]
            f0 = 2 * DH * (h // 2)
            wb, wa = f0 // T, (f0 + 2 * DH - 1) // T
            win = (wb if wa == wb else NG + wa,)
            if (i, h) not in qws:
                qws[i, h] = q_weights(i, h)
            if j < i:
                keep(n, 0, _nn(_ld(k_s, win, t0 + T * j, T), qws[i, h]))
                return
            keep(n, 0, _nn(_ld(k_s, win, t0 + T * j, 32), qws[i, h]) + mask_s[0:32, :])
            if h % 2 == 0:
                ksp[i] = k_split(win[0], i, h // 2)
            sp = _nn(ksp[i], q_split(i, h))
            keep(n, 32, sp + mask_s[32:64, :])
            keep(n, 96, pltpu.roll(sp, 96, 1) + mask_s[96:T, :])
            if h % 2 == 0:
                sh = _nn(_ld(k_s, win, t0 + T * j + 64, 32), q_shared(i, h // 2))
                keep(n, 64, pltpu.roll(sh, 64, 1) + mask_s[64:96, :])
                keep(n + i + 1, 64, sh + mask_s[64:96, :])

        def probs(n):
            i, h, j = tiles[n]
            if (i, h) not in fin:
                fin[i, h] = jnp.max(mx.pop((i, h)), axis=0, keepdims=True)
            pvals[n] = jnp.exp2(s_ring[n % RING][zeros[0]] - fin[i, h]).astype(BF)

        def values(n):
            i, h, j = tiles[n]
            base = (h // 2) * 2 * DH + (h % 2) * 16
            vv = v_s[NQ * s + j, base:base + 24, :]
            if h % 2 == 0:
                vv = jnp.concatenate([vv[:16], jnp.where(sub8 < 4, vv[16:], 1.0)], axis=0)
            else:
                vv = jnp.concatenate([jnp.where(sub8 >= 4, vv[:8], 1.0), vv[8:]], axis=0)
            o = _nn(vv, pvals.pop(n))
            acc[i, h] = o if j == 0 else acc[i, h] + o
            if j == i:
                a = acc.pop((i, h))
                den = a[DH:DH + 1] if h % 2 == 0 else a[0:1]
                w_dot = (1.0 - g_s[h:h + 1, :]) / den
                w_mem = rden_s[NQ * s + i, h:h + 1, :]
                o = a * w_dot + num_s[s, i, base:base + 24, :] * w_mem
                if h % 2 == 0:
                    ot_s[i][0, base:base + 16, :] = o[:16]
                    held[i] = o[16:]
                else:
                    mid = jnp.where(sub8 < 4, held.pop(i), o[:8])
                    ot_s[i][0, base:base + 24, :] = jnp.concatenate([mid, o[8:]], axis=0)

        def out_proj(i):
            ot = jnp.concatenate([ot_s[i][zeros[1], T * w:T * (w + 1), :].T for w in range(NG)],
                                 axis=1)
            wo = jnp.concatenate([_ld(wo_v, (c,), 0, D) for c in range(NG)], axis=1)
            yb_s[s, T * i:T * (i + 1), :] = _nn(ot.astype(BF), wo).astype(BF)

        n = len(tiles)
        todo = list(OUT_ORDER)
        for tt in range(0, n + LAG_EXP + LAG_PV, STEP):
            for fn, lag in ((logits, 0), (probs, LAG_EXP), (values, LAG_EXP + LAG_PV)):
                for k in range(tt - lag, tt - lag + STEP):
                    if 0 <= k < n:
                        fn(k)
            if len(todo) == NQ and tt + STEP >= n:
                out_proj(todo.pop(0))
        for i in todo:
            if i == NQ - 1:
                cp_yb(s, 0).start()
            out_proj(i)
        cp_yb(s, 1).start()
        return carry

    lax.fori_loop(0, NSEG, segment, 0)

    _wait(cp_conv(NG + 1) + [cp_ya(g) for g in range(NG)])
    _wait([cp_yb(s, part) for s in range(NSEG) for part in range(2)])


@jax.jit
def pallas_concat_heads__ssm_conv_h3__memory_aug_infini_attn__prompt_kernel(
    A_q, A_k, A_v, A_shift_k, A_ssm_k, A_ssm_D, B_x, B_wq, B_wk, B_wv, B_wo, B_beta,
):
    scratch = _scratch()

    def body(*refs):
        _kernel(*refs[:14], **dict(zip(scratch, refs[14:])))

    hbm = pl.BlockSpec(memory_space=pl.ANY)
    out = pl.pallas_call(
        body,
        out_shape=jax.ShapeDtypeStruct((S, 2 * D), BF),
        in_specs=[hbm] * 13,
        out_specs=hbm,
        scratch_shapes=list(scratch.values()),
        compiler_params=pltpu.CompilerParams(vmem_limit_bytes=100 * 1024 * 1024),
        name="h3_infini",
    )(A_q.reshape(S, D), A_k.reshape(S, D), A_v.reshape(S, D), A_shift_k.T, A_ssm_k, A_ssm_D,
      B_x.reshape(S, D), B_wq, B_wk, B_wv, B_wo, B_beta, _DFT)
    return out.reshape(1, S, 2 * D)
```

```python
import jax
import jax.numpy as jnp
import numpy as np
from jax import lax
import jax.experimental.pallas as pl
import jax.experimental.pallas.tpu as pltpu

BF = jnp.bfloat16
F32 = jnp.float32
U32 = jnp.uint32
I32 = jnp.int32

S = 2048
D = 640
H = 32
DH = 20
NSEG = 4
L = S // NSEG
T = 128
NB = S // T
NQ = L // T
NG = D // T
LOG2E = 1.4426950408889634
QSCALE = DH ** -0.5 * LOG2E
NEG = -1e9 * LOG2E

PRE = 5
LEAD = 3
NSET = 4
RING = 32
LAG_EXP = 12
LAG_PV = 4
STEP = 4
Q_GROUPS = ((2, 1), (3, 0))
OUT_ORDER = (2, 1, 0, 3)


def _dft_matrices():
    theta = (0.5 * np.pi + 2.0 * np.pi * np.arange(T)) / T
    ang = theta[:, None] * np.arange(T)[None, :]
    f = np.stack([np.cos(ang).reshape(NB, 8, T), np.sin(ang).reshape(NB, 8, T)], axis=1)
    f = f.reshape(2 * T, T)
    g = (f.T / T).reshape(T, 2, T).transpose(1, 0, 2).reshape(2 * T, T)
    return np.concatenate([f, g], axis=0).astype(BF)


_DFT = _dft_matrices()


_H0 = [(T * w) // DH for w in range(NG)]
_H1 = [(T * w + T - 1) // DH for w in range(NG)]
_R0 = [(DH * h) // 8 * 8 for h in _H0]
_R1 = [-(-(DH * (h + 1)) // 8) * 8 for h in _H1]


def _phi(t):
    return jnp.where(t > 0, t + 1.0, jnp.exp(t))


def _head_of(idx):
    return (idx * 3277) >> 16


def _ld(ref, idx, r0, n):
    if isinstance(r0, int):
        rows = pl.ds(r0 // 2, n // 2)
    else:
        rows = pl.ds(pl.multiple_of(r0 // 2, 8), n // 2)
    return pltpu.bitcast(ref.bitcast(U32)[(*idx, rows, slice(None))], BF)


def _nn(a, b):
    return lax.dot_general(a, b, (((1,), (0,)), ((), ())), preferred_element_type=F32)


def _nt(a, b):
    return lax.dot_general(a, b, (((1,), (1,)), ((), ())), preferred_element_type=F32)


def _block_conv(u, k, zs):
    h = NB // 2
    us, ks = [u(a, zs[0]) for a in range(h)], [k(j, zs[0]) for j in range(h)]
    out = []
    for c in range(h):
        acc = us[c] * ks[0]
        for j in range(1, c + 1):
            acc = acc + us[c - j] * ks[j]
        out.append(acc)
    us, ks = [u(a, zs[1]) for a in range(h)], {j: k(j, zs[1]) for j in range(1, NB)}
    hi = []
    for c in range(h, NB):
        acc = us[0] * ks[c]
        for a in range(1, h):
            acc = acc + us[a] * ks[c - a]
        hi.append(acc)
    us, ks = [u(h + a, zs[2]) for a in range(h)], [k(j, zs[2]) for j in range(h)]
    for c in range(h):
        acc = hi[c]
        for j in range(c + 1):
            acc = acc + us[c - j] * ks[j]
        out.append(acc)
    return out


def _start(copies, priority=0):
    for c in copies:
        c.start(priority=priority)


def _wait(copies):
    for c in copies:
        c.wait()


def _scratch():
    vm = pltpu.VMEM
    return dict(
        wo_v=vm((NG, D, T), BF),
        k_s=vm((2 * NG, S, T), BF),
        q_s=vm((NB, D, T), BF),
        v_s=vm((NB, D, T), F32),
        num_s=vm((NSEG, NQ, D, T), F32),
        rden_s=vm((NB, H, T), F32),
        yb_s=vm((NSEG, L, D), BF),
        mask_s=vm((T, T), F32),
        g_s=vm((H, T), F32),
        **{f"ot{i}": vm((1, D, T), F32) for i in range(NQ)},
        **{f"sr{i}": vm((1, T, T), F32) for i in range(RING)},
        aq_v=vm((NG + 2, S, T), BF),
        ak_v=vm((NG + 2, S, T), BF),
        av_v=vm((NG + 2, S, T), BF),
        fk_v=vm((NG + 2, T, S), BF),
        x_v=vm((NG, S, T), BF),
        wq_v=vm((NG, D, T), BF),
        wk_v=vm((NG, D, T), BF),
        wv_v=vm((NG, D, T), BF),
        dft_v=vm((4 * T, T), BF),
        wt_s=vm((NG, NG, 2 * T, T), BF),
        kv_s=vm((S, T), BF),
        uf_s=vm((NB, 2 * T, T), F32),
        kf_s=vm((NB, 2 * T, T), F32),
        us_s=vm((NB, T, T), F32),
        ks_s=vm((NB, T, T), F32),
        z_s=vm((NB, 2 * T, T), BF),
        ya_s=vm((NG, S, T), BF),
        pk_s=vm((NG, S, T), BF),
        pq_s=vm((NB, D, T), BF),
        par_s=vm((NG, 5, 8, T), F32),
        **{f"tr{i}": vm((1, NB, 8, T), F32) for i in range(2 * NSET)},
        sk_v=vm((4, D), BF),
        dd_v=vm((D,), BF),
        beta_v=vm((H,), BF),
        zero_s=pltpu.SMEM((16,), I32),
        sem_s=pltpu.SemaphoreType.DMA((2 + 2 * NG,)),
        sem_g=pltpu.SemaphoreType.DMA((NG + 2,)),
        sem_x=pltpu.SemaphoreType.DMA((2,)),
        sem_out=pltpu.SemaphoreType.DMA((NG + 2 * NSEG,)),
    )


def _kernel(aq_hbm, ak_hbm, av_hbm, sk_hbm, fk_hbm, dd_hbm, x_hbm, wq_hbm, wk_hbm, wv_hbm,
            wo_hbm, beta_hbm, dft_hbm, out_hbm, *, aq_v, ak_v, av_v, fk_v, x_v, wq_v, wk_v, wv_v,
            wo_v, sk_v, dd_v, beta_v, dft_v, wt_s, kv_s, uf_s, kf_s, us_s, ks_s, z_s, ya_s, k_s, q_s, v_s,
            pk_s, pq_s, num_s, rden_s, yb_s, mask_s, par_s, g_s, zero_s, sem_s, sem_g, sem_x,
            sem_out, **rings):
    ot_s = [rings[f"ot{i}"] for i in range(NQ)]
    s_ring = [rings[f"sr{i}"] for i in range(RING)]
    t_ring = [rings[f"tr{i}"] for i in range(2 * NSET)]

    def col(g):
        return pl.ds(g * T if isinstance(g, int) else pl.multiple_of(g * T, T), T)

    def cp_small():
        return [pltpu.make_async_copy(src, dst, sem_s.at[0]) for src, dst in
                ((sk_hbm, sk_v), (dd_hbm, dd_v), (beta_hbm, beta_v), (dft_hbm, dft_v))]

    def cp_wo():
        return [pltpu.make_async_copy(wo_hbm.at[:, col(w)], wo_v.at[w], sem_s.at[1])
                for w in range(NG)]

    def cp_w(windows):
        cs = []
        for g in windows:
            cs.append(pltpu.make_async_copy(wk_hbm.at[:, col(g)], wk_v.at[g], sem_s.at[2 + g]))
            cs += [pltpu.make_async_copy(src.at[:, col(g)], dst.at[g], sem_s.at[2 + NG + g])
                   for src, dst in ((wq_hbm, wq_v), (wv_hbm, wv_v))]
        return cs

    def cp_x(part):
        lo, hi = ((0, PRE), (PRE, NB))[part]
        rows = pl.ds(T * lo, T * (hi - lo))
        return [pltpu.make_async_copy(x_hbm.at[rows, col(w)], x_v.at[w, rows], sem_x.at[part])
                for w in range(NG)]

    def cp_conv(g):
        src = min(g, NG - 1) if isinstance(g, int) else jnp.minimum(g, NG - 1)
        return [pltpu.make_async_copy(fk_hbm.at[col(src), :], fk_v.at[g], sem_g.at[g])] + [
            pltpu.make_async_copy(a.at[:, col(src)], dst.at[g], sem_g.at[g])
            for a, dst in ((ak_hbm, ak_v), (av_hbm, av_v), (aq_hbm, aq_v))]

    def cp_ya(g):
        return pltpu.make_async_copy(ya_s.at[g], out_hbm.at[:, col(g)], sem_out.at[g])

    def cp_yb(s, part):
        lo, n = ((0, L - T), (L - T, T))[part]
        r0 = s * L + lo if isinstance(s, int) else pl.multiple_of(s * L + lo, T)
        return pltpu.make_async_copy(yb_s.at[s, pl.ds(lo, n)], out_hbm.at[pl.ds(r0, n), D:2 * D],
                                     sem_out.at[NG + 2 * s + part])

    _start(cp_x(0) + cp_w((0,)))
    _start(cp_x(1) + cp_conv(0), priority=1)

    for i in range(16):
        zero_s[i] = 0
    r_i = lax.broadcasted_iota(I32, (T, T), 0)
    c_i = lax.broadcasted_iota(I32, (T, T), 1)
    mask_s[...] = jnp.where(r_i <= c_i, 0.0, NEG)

    def x_tile(t):
        return jnp.concatenate([_ld(x_v, (c,), T * t, T) for c in range(NG)], axis=1)

    def proj_k(g, t, z):
        rows = slice(T * t, T * (t + 1))
        k = _nn(x_tile(t), _ld(wk_v, (g,), 0, D))
        k_s[g, rows, :] = k.astype(BF)
        if t < NB - NQ:
            pk_s[g, rows, :] = _phi(k).astype(BF)

    def straddle(g, t, z):
        words = slice(T * t // 2, T * (t + 1) // 2)
        gp = g - 1 if isinstance(g, int) else jnp.maximum(g - 1, 0)
        ku = k_s.bitcast(U32)
        ku[NG + g, words, :] = jnp.where(c_i[:T // 2] < 64, ku[g + z, words, :], ku[gp + z, words, :])

    def proj_qv(g, t, z):
        wt = jnp.concatenate([_ld(wt_s, (g + z, c), 0, 2 * T) for c in range(NG)], axis=1)
        qv = _nt(wt, x_tile(t))
        q = qv[:T]
        q_s[t, col(g), :] = (q * QSCALE).astype(BF)
        if t >= NQ:
            pq_s[t, col(g), :] = _phi(q).astype(BF)
        v_s[t, col(g), :] = qv[T:]

    def project_first(windows, z):
        for g in windows:
            for c in range(NG):
                wt_s[g, c, 0:T, :] = _ld(wq_v, (g,), T * c, T).T
                wt_s[g, c, T:2 * T, :] = _ld(wv_v, (g,), T * c, T).T
        jobs = [(g, t) for g in windows for t in range(PRE)]
        for fn in (proj_k, proj_qv):
            for g, t in jobs:
                fn(g, t, z)
        for g, t in jobs:
            if g:
                straddle(g, t, z)

    _wait(cp_x(0) + cp_w((0,)))
    z0 = zero_s[0]
    num_s[0] = jnp.zeros((NQ, D, T), F32)
    rden_s[0:NQ] = jnp.zeros((NQ, H, T), F32)
    _start(cp_w((1,)) + cp_small())
    project_first((0,), z0)
    _start(cp_w((2, 3, 4)))
    _wait(cp_w((1,)) + cp_small())
    taps = sk_v[...].astype(F32)
    dvec = dd_v[...].astype(F32).reshape(1, D)
    for g in range(NG):
        for j in range(4):
            par_s[g, j] = jnp.broadcast_to(taps[j:j + 1, T * g:T * (g + 1)], (8, T))
        par_s[g, 4] = jnp.broadcast_to(dvec[:, T * g:T * (g + 1)], (8, T))
    gate = jax.nn.sigmoid(beta_v[...].astype(F32).reshape(1, H)).astype(BF).astype(F32)
    hr = lax.broadcasted_iota(I32, (H, H), 0)
    hc = lax.broadcasted_iota(I32, (H, H), 1)
    gcol = jnp.sum(jnp.where(hr == hc, jnp.broadcast_to(gate, (H, H)), 0.0), axis=1, keepdims=True)
    g_s[...] = jnp.broadcast_to(gcol, (H, T))
    project_first((1,), z0)
    _wait(cp_w((2, 3, 4)))
    project_first((2, 3, 4), z0)
    _wait(cp_x(1) + cp_conv(0))
    _start(cp_conv(1))
    _start(cp_wo(), priority=1)

    def group(g, carry):
        zeros = [zero_s[i] for i in range(9)]

        def re_plus_im(f):
            return jnp.concatenate([f[16 * s:16 * s + 8] + f[16 * s + 8:16 * s + 16]
                                    for s in range(NB)], axis=0)

        def filt(j):
            f = _nt(_ld(dft_v, (), 0, 2 * T), fk_v[g, :, T * j:T * (j + 1)])
            kf_s[j] = f
            ks_s[j] = re_plus_im(f)

        def kv(a):
            cur = _ld(ak_v, (g,), T * a, T).astype(F32)
            if a == 0:
                prev = jnp.zeros((8, T), F32)
            else:
                prev = _ld(ak_v, (g,), T * a - 16, 16).astype(F32)[8:]
            ext = jnp.concatenate([prev, cur], axis=0)
            acc = cur * par_s[g, 0][0:1]
            for j in range(1, 4):
                acc = acc + ext[8 - j:8 - j + T] * par_s[g, j][0:1]
            u = (acc * _ld(av_v, (g,), T * a, T).astype(F32)).astype(BF)
            kv_s[T * a:T * (a + 1), :] = u
            f = _nn(_ld(dft_v, (), 0, 2 * T), u)
            uf_s[a] = f
            us_s[a] = re_plus_im(f)

        def slab(s):
            re, im = slice(16 * s, 16 * s + 8), slice(16 * s + 8, 16 * s + 16)
            both = slice(8 * s, 8 * s + 8)
            rr_s, ii_s = t_ring[2 * (s % NSET)], t_ring[2 * (s % NSET) + 1]
            for part, dst in ((re, rr_s), (im, ii_s)):
                t = _block_conv(lambda a, z: uf_s[a + z, part, :],
                                lambda j, z: kf_s[j + z, part, :], zeros[0:3])
                for c in range(NB):
                    dst[0, c] = t[c]
            t = _block_conv(lambda a, z: us_s[a + z, both, :],
                            lambda j, z: ks_s[j + z, both, :], zeros[3:6])
            pr = pi = None
            for c in range(NB):
                rr, ii = rr_s[zeros[6], c], ii_s[zeros[6], c]
                wr, wi = rr - ii, t[c] - rr - ii
                zr, zi = (wr, wi) if c == 0 else (wr + pi, wi - pr)
                pr, pi = wr, wi
                z_s[c, 16 * s:16 * s + 16, :] = jnp.concatenate([zr, zi], axis=0).astype(BF)

        def inv(c):
            z = zeros[7]
            y = (_nn(_ld(dft_v, (), 2 * T, T), _ld(z_s, (c + z,), 0, T))
                 + _nn(_ld(dft_v, (), 3 * T, T), _ld(z_s, (c + z,), T, T)))
            y = y + _ld(kv_s, (), T * c + z, T).astype(F32) * par_s[g, 4][0:1]
            ya_s[g, T * c:T * (c + 1), :] = (_ld(aq_v, (g,), T * c, T).astype(F32) * y).astype(BF)

        for j in range(NB + LEAD):
            if j < NB:
                filt(j)
            if j >= LEAD:
                kv(j - LEAD)
        for t in range(PRE, NB):
            proj_k(g, t, zeros[8])
            proj_qv(g, t, zeros[8])
            if t > PRE:
                straddle(g, t - 1, zeros[8])
        straddle(g, NB - 1, zeros[8])
        for s in range(NB):
            slab(s)
        for c in range(NB):
            inv(c)
        _start(cp_conv(g + 2))
        _wait(cp_conv(g + 1))
        return carry

    lax.fori_loop(0, NG, group, 0)

    gcolv = g_s[...]
    mem = [None] * NG
    for s in range(NSEG - 1):
        lhs = []
        for w in range(NG):
            n = _R1[w] - _R0[w]
            vv = jnp.concatenate([v_s[NQ * s + i, _R0[w]:_R1[w], :] for i in range(NQ)], axis=1)
            vv = jnp.concatenate([vv, jnp.ones((8, L), F32)], axis=0)
            upd = _nn(vv, _ld(pk_s, (w,), L * s, L))
            mem[w] = upd if mem[w] is None else mem[w] + upd
            rh = _head_of(lax.broadcasted_iota(I32, (n, T), 0) + _R0[w])
            ch = _head_of(lax.broadcasted_iota(I32, (n, T), 1) + T * w)
            zh = lax.broadcasted_iota(I32, (8, T), 0) + _H0[w]
            ch8 = _head_of(lax.broadcasted_iota(I32, (8, T), 1) + T * w)
            lhs.append(jnp.concatenate([jnp.where(rh == ch, mem[w][:n], 0.0),
                                        jnp.where(zh == ch8, mem[w][n:], 0.0)], axis=0))
        for i in range(NQ):
            t = NQ * (s + 1) + i
            res = [_nn(lhs[w], _ld(pq_s, (t,), T * w, T)) for w in range(NG)]
            den = None
            for w in range(NG):
                lo = _R0[w] if w == 0 else _R1[w - 1]
                hi = _R1[w] if w == NG - 1 else _R0[w + 1]
                num_s[s + 1, i, lo:hi, :] = res[w][lo - _R0[w]:hi - _R0[w]]
                if w + 1 < NG:
                    num_s[s + 1, i, hi:_R1[w], :] = (res[w][hi - _R0[w]:_R1[w] - _R0[w]]
                                                     + res[w + 1][:_R1[w] - hi])
                part = jnp.concatenate(
                    ([jnp.zeros((_H0[w], T), F32)] if _H0[w] else [])
                    + [res[w][_R1[w] - _R0[w]:], jnp.zeros((H - _H0[w], T), F32)], axis=0)[:H]
                den = part if den is None else den + part
            rden_s[t] = gcolv / (den + 1e-6)

    _wait(cp_wo())
    _start([cp_ya(g) for g in range(NG)])

    tiles = [(i, h, j) for grp in Q_GROUPS for m in range(H // 2) for i in grp
             for h in (2 * m, 2 * m + 1) for j in range(i + 1)]

    def segment(s, carry):
        zeros = [zero_s[9 + i] for i in range(2)]
        sub8 = lax.broadcasted_iota(I32, (8, T), 0)
        lane8 = lax.broadcasted_iota(I32, (8, T), 1)
        t0 = pl.multiple_of(s * L, L)
        qws, mx, pvals, acc, fin, held, ksp = {}, {}, {}, {}, {}, {}, {}

        def q_blocks(i, h):
            f0 = DH * h
            for b in (f0 // 16, f0 // 16 + 1):
                blk = q_s.bitcast(U32)[NQ * s + i, 8 * b:8 * b + 8, :]
                lo, hi = f0 // 2 - 8 * b, (f0 + DH) // 2 - 8 * b
                if lo > 0:
                    blk = jnp.where(sub8 >= lo, blk, jnp.uint32(0))
                if hi < 8:
                    blk = jnp.where(sub8 < hi, blk, jnp.uint32(0))
                yield b, blk

        def q_weights(i, h):
            blocks = [jnp.zeros((8, T), U32)] * 8
            for b, blk in q_blocks(i, h):
                blocks[b % 8] = blk
            return pltpu.bitcast(jnp.concatenate(blocks, axis=0), BF)

        def q_shared(i, m):
            f0 = 2 * DH * m
            blocks = [jnp.zeros((8, T), U32)] * 8
            for b in range(f0 // 16, (f0 + 2 * DH - 1) // 16 + 1):
                blk = q_s.bitcast(U32)[NQ * s + i, 8 * b:8 * b + 8, :]
                row = sub8 + 8 * b - f0 // 2
                in_a = (row >= 0) & (row < DH // 2) & (lane8 < 64)
                in_b = (row >= DH // 2) & (row < DH) & (lane8 >= 64)
                blocks[b % 8] = jnp.where(in_a, pltpu.roll(blk, 64, 1),
                                          jnp.where(in_b, blk, jnp.uint32(0)))
            return pltpu.bitcast(jnp.concatenate(blocks, axis=0), BF)

        def q_split(i, h):
            blocks = [jnp.zeros((8, T), U32)] * 8
            for b, blk in q_blocks(i, h):
                blocks[b % 8] = jnp.where(lane8 >= 32, blk, jnp.uint32(0))
                blocks[(b + 4) % 8] = jnp.where(lane8 < 32, pltpu.roll(blk, 32, 1), jnp.uint32(0))
            return pltpu.bitcast(jnp.concatenate(blocks, axis=0), BF)

        def k_split(win, i, m):
            ku = k_s.bitcast(U32)
            r0 = pl.multiple_of((t0 + T * i) // 2, 8)
            first = ku[win, pl.ds(r0 + 16, 16), :]
            second = pltpu.roll(ku[win, pl.ds(r0 + 48, 16), :], 64, 1)
            lane = lax.broadcasted_iota(I32, (16, T), 1)
            return pltpu.bitcast(jnp.where(((lane - 2 * DH * m) & (T - 1)) < 64, first, second), BF)

        def keep(n, r0, sc):
            i, h, _ = tiles[n]
            m8 = jnp.max(sc.reshape(sc.shape[0] // 8, 8, T), axis=0)
            mx[i, h] = m8 if (i, h) not in mx else jnp.maximum(mx[i, h], m8)
            s_ring[n % RING][0, r0:r0 + sc.shape[0], :] = sc

        def logits(n):
            i, h, j = tiles[n]
            f0 = 2 * DH * (h // 2)
            wb, wa = f0 // T, (f0 + 2 * DH - 1) // T
            win = (wb if wa == wb else NG + wa,)
            if (i, h) not in qws:
                qws[i, h] = q_weights(i, h)
            if j < i:
                keep(n, 0, _nn(_ld(k_s, win, t0 + T * j, T), qws[i, h]))
                return
            keep(n, 0, _nn(_ld(k_s, win, t0 + T * j, 32), qws[i, h]) + mask_s[0:32, :])
            if h % 2 == 0:
                ksp[i] = k_split(win[0], i, h // 2)
            sp = _nn(ksp[i], q_split(i, h))
            keep(n, 32, sp + mask_s[32:64, :])
            keep(n, 96, pltpu.roll(sp, 96, 1) + mask_s[96:T, :])
            if h % 2 == 0:
                sh = _nn(_ld(k_s, win, t0 + T * j + 64, 32), q_shared(i, h // 2))
                keep(n, 64, pltpu.roll(sh, 64, 1) + mask_s[64:96, :])
                keep(n + i + 1, 64, sh + mask_s[64:96, :])

        def probs(n):
            i, h, j = tiles[n]
            if (i, h) not in fin:
                fin[i, h] = jnp.max(mx.pop((i, h)), axis=0, keepdims=True)
            pvals[n] = jnp.exp2(s_ring[n % RING][zeros[0]] - fin[i, h]).astype(BF)

        def values(n):
            i, h, j = tiles[n]
            base = (h // 2) * 2 * DH + (h % 2) * 16
            vv = v_s[NQ * s + j, base:base + 24, :]
            if h % 2 == 0:
                vv = jnp.concatenate([vv[:16], jnp.where(sub8 < 4, vv[16:], 1.0)], axis=0)
            else:
                vv = jnp.concatenate([jnp.where(sub8 >= 4, vv[:8], 1.0), vv[8:]], axis=0)
            o = _nn(vv, pvals.pop(n))
            acc[i, h] = o if j == 0 else acc[i, h] + o
            if j == i:
                a = acc.pop((i, h))
                den = a[DH:DH + 1] if h % 2 == 0 else a[0:1]
                w_dot = (1.0 - g_s[h:h + 1, :]) / den
                w_mem = rden_s[NQ * s + i, h:h + 1, :]
                o = a * w_dot + num_s[s, i, base:base + 24, :] * w_mem
                if h % 2 == 0:
                    ot_s[i][0, base:base + 16, :] = o[:16]
                    held[i] = o[16:]
                else:
                    mid = jnp.where(sub8 < 4, held.pop(i), o[:8])
                    ot_s[i][0, base:base + 24, :] = jnp.concatenate([mid, o[8:]], axis=0)

        def out_proj(i):
            ot = jnp.concatenate([ot_s[i][zeros[1], T * w:T * (w + 1), :].T for w in range(NG)],
                                 axis=1)
            wo = jnp.concatenate([_ld(wo_v, (c,), 0, D) for c in range(NG)], axis=1)
            yb_s[s, T * i:T * (i + 1), :] = _nn(ot.astype(BF), wo).astype(BF)

        n = len(tiles)
        todo = list(OUT_ORDER)
        for tt in range(0, n + LAG_EXP + LAG_PV, STEP):
            for fn, lag in ((logits, 0), (probs, LAG_EXP), (values, LAG_EXP + LAG_PV)):
                for k in range(tt - lag, tt - lag + STEP):
                    if 0 <= k < n:
                        fn(k)
            if len(todo) == NQ and tt + STEP >= n:
                out_proj(todo.pop(0))
        for i in todo:
            if i == NQ - 1:
                cp_yb(s, 0).start()
            out_proj(i)
        cp_yb(s, 1).start()
        return carry

    lax.fori_loop(0, NSEG, segment, 0)

    _wait(cp_conv(NG + 1) + [cp_ya(g) for g in range(NG)])
    _wait([cp_yb(s, part) for s in range(NSEG) for part in range(2)])


@jax.jit
def pallas_concat_heads__ssm_conv_h3__memory_aug_infini_attn__prompt_kernel(
    A_q, A_k, A_v, A_shift_k, A_ssm_k, A_ssm_D, B_x, B_wq, B_wk, B_wv, B_wo, B_beta,
):
    scratch = _scratch()

    def body(*refs):
        _kernel(*refs[:14], **dict(zip(scratch, refs[14:])))

    hbm = pl.BlockSpec(memory_space=pl.ANY)
    out = pl.pallas_call(
        body,
        out_shape=jax.ShapeDtypeStruct((S, 2 * D), BF),
        in_specs=[hbm] * 13,
        out_specs=hbm,
        scratch_shapes=list(scratch.values()),
        compiler_params=pltpu.CompilerParams(vmem_limit_bytes=100 * 1024 * 1024),
        name="h3_infini",
    )(A_q.reshape(S, D), A_k.reshape(S, D), A_v.reshape(S, D), A_shift_k.T, A_ssm_k, A_ssm_D,
      B_x.reshape(S, D), B_wq, B_wk, B_wv, B_wo, B_beta, _DFT)
    return out.reshape(1, S, 2 * D)
```

```python
import jax
import jax.numpy as jnp
import numpy as np
from jax import lax
import jax.experimental.pallas as pl
import jax.experimental.pallas.tpu as pltpu

BF = jnp.bfloat16
F32 = jnp.float32
U32 = jnp.uint32
I32 = jnp.int32

S = 2048
D = 640
H = 32
DH = 20
NSEG = 4
L = S // NSEG
T = 128
NB = S // T
NQ = L // T
NG = D // T
LOG2E = 1.4426950408889634
QSCALE = DH ** -0.5 * LOG2E
NEG = -1e9 * LOG2E

PRE = 5
LEAD = 3
EARLY = (2, 0, 0, 0)
NSET = 4
RING = 32
LAG_EXP = 12
LAG_PV = 4
STEP = 4
Q_GROUPS = ((2, 1), (3, 0))
OUT_ORDER = (2, 1, 0, 3)


def _dft_matrices():
    theta = (0.5 * np.pi + 2.0 * np.pi * np.arange(T)) / T
    ang = theta[:, None] * np.arange(T)[None, :]
    f = np.stack([np.cos(ang).reshape(NB, 8, T), np.sin(ang).reshape(NB, 8, T)], axis=1)
    f = f.reshape(2 * T, T)
    g = (f.T / T).reshape(T, 2, T).transpose(1, 0, 2).reshape(2 * T, T)
    return np.concatenate([f, g], axis=0).astype(BF)


_DFT = _dft_matrices()


def _phi(t):
    return jnp.where(t > 0, t + 1.0, jnp.exp(t))


def _head_of(idx):
    return (idx * 3277) >> 16


def _ld(ref, idx, r0, n):
    if isinstance(r0, int):
        rows = pl.ds(r0 // 2, n // 2)
    else:
        rows = pl.ds(pl.multiple_of(r0 // 2, 8), n // 2)
    return pltpu.bitcast(ref.bitcast(U32)[(*idx, rows, slice(None))], BF)


def _nn(a, b):
    return lax.dot_general(a, b, (((1,), (0,)), ((), ())), preferred_element_type=F32)


def _nt(a, b):
    return lax.dot_general(a, b, (((1,), (1,)), ((), ())), preferred_element_type=F32)


def _block_conv(u, k, zs):
    h = NB // 2
    us, ks = [u(a, zs[0]) for a in range(h)], [k(j, zs[0]) for j in range(h)]
    out = []
    for c in range(h):
        acc = us[c] * ks[0]
        for j in range(1, c + 1):
            acc = acc + us[c - j] * ks[j]
        out.append(acc)
    us, ks = [u(a, zs[1]) for a in range(h)], {j: k(j, zs[1]) for j in range(1, NB)}
    hi = []
    for c in range(h, NB):
        acc = us[0] * ks[c]
        for a in range(1, h):
            acc = acc + us[a] * ks[c - a]
        hi.append(acc)
    us, ks = [u(h + a, zs[2]) for a in range(h)], [k(j, zs[2]) for j in range(h)]
    for c in range(h):
        acc = hi[c]
        for j in range(c + 1):
            acc = acc + us[c - j] * ks[j]
        out.append(acc)
    return out


def _start(copies, priority=0):
    for c in copies:
        c.start(priority=priority)


def _wait(copies):
    for c in copies:
        c.wait()


def _scratch():
    vm = pltpu.VMEM
    return dict(
        wo_v=vm((NG, D, T), BF),
        k_s=vm((2 * NG, S, T), BF),
        q_s=vm((NB, D, T), BF),
        v_s=vm((NB, D, T), F32),
        num_s=vm((NSEG, NQ, D, T), F32),
        rden_s=vm((NB, H, T), F32),
        yb_s=vm((NSEG, L, D), BF),
        mask_s=vm((T, T), F32),
        g_s=vm((H, T), F32),
        **{f"ot{i}": vm((1, D, T), F32) for i in range(NQ)},
        **{f"sr{i}": vm((1, T, T), F32) for i in range(RING)},
        aq_v=vm((NG + 2, S, T), BF),
        ak_v=vm((NG + 2, S, T), BF),
        av_v=vm((NG + 2, S, T), BF),
        fk_v=vm((NG + 2, T, S), BF),
        x_v=vm((NG, S, T), BF),
        wq_v=vm((NG, D, T), BF),
        wk_v=vm((NG, D, T), BF),
        wv_v=vm((NG, D, T), BF),
        dft_v=vm((4 * T, T), BF),
        wt_s=vm((NG, NG, 2 * T, T), BF),
        kv_s=vm((S, T), BF),
        uf_s=vm((NB, 2 * T, T), F32),
        kf_s=vm((NB, 2 * T, T), F32),
        us_s=vm((NB, T, T), F32),
        ks_s=vm((NB, T, T), F32),
        z_s=vm((NB, 2 * T, T), BF),
        ya_s=vm((NG, S, T), BF),
        pk_s=vm((NG, S, T), BF),
        pq_s=vm((NB, D, T), BF),
        par_s=vm((NG, 5, 8, T), F32),
        **{f"tr{i}": vm((1, NB, 8, T), F32) for i in range(2 * NSET)},
        sk_v=vm((4, D), BF),
        dd_v=vm((D,), BF),
        beta_v=vm((H,), BF),
        zero_s=pltpu.SMEM((16,), I32),
        sem_s=pltpu.SemaphoreType.DMA((2 + 2 * NG,)),
        sem_g=pltpu.SemaphoreType.DMA((NG + 2,)),
        sem_x=pltpu.SemaphoreType.DMA((2,)),
        sem_out=pltpu.SemaphoreType.DMA((NG + 2 * NSEG,)),
    )


def _kernel(aq_hbm, ak_hbm, av_hbm, sk_hbm, fk_hbm, dd_hbm, x_hbm, wq_hbm, wk_hbm, wv_hbm,
            wo_hbm, beta_hbm, dft_hbm, out_hbm, *, aq_v, ak_v, av_v, fk_v, x_v, wq_v, wk_v, wv_v,
            wo_v, sk_v, dd_v, beta_v, dft_v, wt_s, kv_s, uf_s, kf_s, us_s, ks_s, z_s, ya_s, k_s, q_s, v_s,
            pk_s, pq_s, num_s, rden_s, yb_s, mask_s, par_s, g_s, zero_s, sem_s, sem_g, sem_x,
            sem_out, **rings):
    ot_s = [rings[f"ot{i}"] for i in range(NQ)]
    s_ring = [rings[f"sr{i}"] for i in range(RING)]
    t_ring = [rings[f"tr{i}"] for i in range(2 * NSET)]

    def col(g):
        return pl.ds(g * T if isinstance(g, int) else pl.multiple_of(g * T, T), T)

    def cp_small():
        return [pltpu.make_async_copy(src, dst, sem_s.at[0]) for src, dst in
                ((sk_hbm, sk_v), (dd_hbm, dd_v), (beta_hbm, beta_v), (dft_hbm, dft_v))]

    def cp_wo():
        return [pltpu.make_async_copy(wo_hbm.at[:, col(w)], wo_v.at[w], sem_s.at[1])
                for w in range(NG)]

    def cp_w(windows):
        cs = []
        for g in windows:
            cs.append(pltpu.make_async_copy(wk_hbm.at[:, col(g)], wk_v.at[g], sem_s.at[2 + g]))
            cs += [pltpu.make_async_copy(src.at[:, col(g)], dst.at[g], sem_s.at[2 + NG + g])
                   for src, dst in ((wq_hbm, wq_v), (wv_hbm, wv_v))]
        return cs

    def cp_x(part):
        lo, hi = ((0, PRE), (PRE, NB))[part]
        rows = pl.ds(T * lo, T * (hi - lo))
        return [pltpu.make_async_copy(x_hbm.at[rows, col(w)], x_v.at[w, rows], sem_x.at[part])
                for w in range(NG)]

    def cp_conv(g):
        src = min(g, NG - 1) if isinstance(g, int) else jnp.minimum(g, NG - 1)
        return [pltpu.make_async_copy(fk_hbm.at[col(src), :], fk_v.at[g], sem_g.at[g])] + [
            pltpu.make_async_copy(a.at[:, col(src)], dst.at[g], sem_g.at[g])
            for a, dst in ((ak_hbm, ak_v), (av_hbm, av_v), (aq_hbm, aq_v))]

    def cp_ya(g):
        return pltpu.make_async_copy(ya_s.at[g], out_hbm.at[:, col(g)], sem_out.at[g])

    def cp_yb(s, part):
        lo, n = ((0, L - T), (L - T, T))[part]
        r0 = s * L + lo if isinstance(s, int) else pl.multiple_of(s * L + lo, T)
        return pltpu.make_async_copy(yb_s.at[s, pl.ds(lo, n)], out_hbm.at[pl.ds(r0, n), D:2 * D],
                                     sem_out.at[NG + 2 * s + part])

    _start(cp_x(0) + cp_w((0,)))
    _start(cp_x(1) + cp_conv(0), priority=1)

    for i in range(16):
        zero_s[i] = 0
    r_i = lax.broadcasted_iota(I32, (T, T), 0)
    c_i = lax.broadcasted_iota(I32, (T, T), 1)
    mask_s[...] = jnp.where(r_i <= c_i, 0.0, NEG)

    def x_tile(t):
        return jnp.concatenate([_ld(x_v, (c,), T * t, T) for c in range(NG)], axis=1)

    def proj_k(g, t, z):
        rows = slice(T * t, T * (t + 1))
        k = _nn(x_tile(t), _ld(wk_v, (g,), 0, D))
        k_s[g, rows, :] = k.astype(BF)
        if t < NB - NQ:
            pk_s[g, rows, :] = _phi(k).astype(BF)

    def straddle(g, t, z):
        words = slice(T * t // 2, T * (t + 1) // 2)
        gp = g - 1 if isinstance(g, int) else jnp.maximum(g - 1, 0)
        ku = k_s.bitcast(U32)
        ku[NG + g, words, :] = jnp.where(c_i[:T // 2] < 64, ku[g + z, words, :], ku[gp + z, words, :])

    def proj_qv(g, t, z):
        wt = jnp.concatenate([_ld(wt_s, (g + z, c), 0, 2 * T) for c in range(NG)], axis=1)
        qv = _nt(wt, x_tile(t))
        q = qv[:T]
        q_s[t, col(g), :] = (q * QSCALE).astype(BF)
        pq_s[t, col(g), :] = _phi(q).astype(BF)
        v_s[t, col(g), :] = qv[T:]

    def project_first(windows, z):
        for g in windows:
            for c in range(NG):
                wt_s[g, c, 0:T, :] = _ld(wq_v, (g,), T * c, T).T
                wt_s[g, c, T:2 * T, :] = _ld(wv_v, (g,), T * c, T).T
        jobs = [(g, t) for g in windows for t in range(PRE)]
        for fn in (proj_k, proj_qv):
            for g, t in jobs:
                fn(g, t, z)
        for g, t in jobs:
            if g:
                straddle(g, t, z)

    _wait(cp_x(0) + cp_w((0,)))
    z0 = zero_s[0]
    _start(cp_w((1,)) + cp_small())
    project_first((0,), z0)
    _start(cp_w((2, 3, 4)))
    _wait(cp_w((1,)) + cp_small())
    taps = sk_v[...].astype(F32)
    dvec = dd_v[...].astype(F32).reshape(1, D)
    for g in range(NG):
        for j in range(4):
            par_s[g, j] = jnp.broadcast_to(taps[j:j + 1, T * g:T * (g + 1)], (8, T))
        par_s[g, 4] = jnp.broadcast_to(dvec[:, T * g:T * (g + 1)], (8, T))
    gate = jax.nn.sigmoid(beta_v[...].astype(F32).reshape(1, H)).astype(BF).astype(F32)
    hr = lax.broadcasted_iota(I32, (H, H), 0)
    hc = lax.broadcasted_iota(I32, (H, H), 1)
    gcol = jnp.sum(jnp.where(hr == hc, jnp.broadcast_to(gate, (H, H)), 0.0), axis=1, keepdims=True)
    g_s[...] = jnp.broadcast_to(gcol, (H, T))
    project_first((1,), z0)
    _wait(cp_w((2, 3, 4)))
    project_first((2, 3, 4), z0)
    _wait(cp_x(1) + cp_conv(0))
    _start(cp_conv(1))
    _start(cp_wo(), priority=1)

    def group(g, carry):
        zeros = [zero_s[i] for i in range(9)]

        def re_plus_im(f):
            return jnp.concatenate([f[16 * s:16 * s + 8] + f[16 * s + 8:16 * s + 16]
                                    for s in range(NB)], axis=0)

        def filt(j):
            f = _nt(_ld(dft_v, (), 0, 2 * T), fk_v[g, :, T * j:T * (j + 1)])
            kf_s[j] = f
            ks_s[j] = re_plus_im(f)

        def kv(a):
            cur = _ld(ak_v, (g,), T * a, T).astype(F32)
            if a == 0:
                prev = jnp.zeros((8, T), F32)
            else:
                prev = _ld(ak_v, (g,), T * a - 16, 16).astype(F32)[8:]
            ext = jnp.concatenate([prev, cur], axis=0)
            acc = cur * par_s[g, 0][0:1]
            for j in range(1, 4):
                acc = acc + ext[8 - j:8 - j + T] * par_s[g, j][0:1]
            u = (acc * _ld(av_v, (g,), T * a, T).astype(F32)).astype(BF)
            kv_s[T * a:T * (a + 1), :] = u
            f = _nn(_ld(dft_v, (), 0, 2 * T), u)
            uf_s[a] = f
            us_s[a] = re_plus_im(f)

        def slab(s):
            re, im = slice(16 * s, 16 * s + 8), slice(16 * s + 8, 16 * s + 16)
            both = slice(8 * s, 8 * s + 8)
            rr_s, ii_s = t_ring[2 * (s % NSET)], t_ring[2 * (s % NSET) + 1]
            for part, dst in ((re, rr_s), (im, ii_s)):
                t = _block_conv(lambda a, z: uf_s[a + z, part, :],
                                lambda j, z: kf_s[j + z, part, :], zeros[0:3])
                for c in range(NB):
                    dst[0, c] = t[c]
            t = _block_conv(lambda a, z: us_s[a + z, both, :],
                            lambda j, z: ks_s[j + z, both, :], zeros[3:6])
            pr = pi = None
            for c in range(NB):
                rr, ii = rr_s[zeros[6], c], ii_s[zeros[6], c]
                wr, wi = rr - ii, t[c] - rr - ii
                zr, zi = (wr, wi) if c == 0 else (wr + pi, wi - pr)
                pr, pi = wr, wi
                z_s[c, 16 * s:16 * s + 16, :] = jnp.concatenate([zr, zi], axis=0).astype(BF)

        def inv(c):
            z = zeros[7]
            y = (_nn(_ld(dft_v, (), 2 * T, T), _ld(z_s, (c + z,), 0, T))
                 + _nn(_ld(dft_v, (), 3 * T, T), _ld(z_s, (c + z,), T, T)))
            y = y + _ld(kv_s, (), T * c + z, T).astype(F32) * par_s[g, 4][0:1]
            ya_s[g, T * c:T * (c + 1), :] = (_ld(aq_v, (g,), T * c, T).astype(F32) * y).astype(BF)

        for j in range(NB + LEAD):
            if j < NB:
                filt(j)
            if j >= LEAD:
                kv(j - LEAD)
        for t in range(PRE, NB):
            proj_k(g, t, zeros[8])
            proj_qv(g, t, zeros[8])
            if t > PRE:
                straddle(g, t - 1, zeros[8])
        straddle(g, NB - 1, zeros[8])
        for s in range(NB):
            slab(s)
        for c in range(NB):
            inv(c)
        _start(cp_conv(g + 2))
        _wait(cp_conv(g + 1))
        return carry

    lax.fori_loop(0, NG, group, 0)

    gcolv = g_s[...]
    span = 6 * DH
    starts = list(range(0, D, span))
    mem = [jnp.zeros((min(span, D - f0), T), F32) for f0 in starts]
    zsum = [jnp.zeros((8, T), F32) for f0 in starts]

    def pk_window(s, f0):
        w, shift = divmod(f0, T)
        words = slice(L * s // 2, L * (s + 1) // 2)
        pu = pk_s.bitcast(U32)
        val = pu[w, words, :]
        if shift:
            val = pltpu.roll(val, T - shift, 1)
            if w + 1 < NG:
                low = lax.broadcasted_iota(I32, (L // 2, T), 1) < T - shift
                val = jnp.where(low, val, pltpu.roll(pu[w + 1, words, :], T - shift, 1))
        return pltpu.bitcast(val, BF)

    for s in range(NSEG):
        lhs = []
        for f0, m, zs in zip(starts, mem, zsum):
            rh = _head_of(lax.broadcasted_iota(I32, m.shape, 0) + f0)
            ch = _head_of(lax.broadcasted_iota(I32, m.shape, 1) + f0)
            zh = lax.broadcasted_iota(I32, (8, T), 0) + f0 // DH
            ch8 = _head_of(lax.broadcasted_iota(I32, (8, T), 1) + f0)
            z = jnp.broadcast_to(jnp.sum(zs, axis=0, keepdims=True), (8, T))
            lhs.append(jnp.concatenate([jnp.where(rh == ch, m, 0.0),
                                        jnp.where(zh == ch8, z, 0.0)], axis=0))

        def read_out(i):
            t = NQ * s + i
            den = []
            for f0, m in zip(starts, lhs):
                rows = m.shape[0] - 8
                pq = pq_s.bitcast(U32)[t, f0 // 2:min(f0 + T, D) // 2, :]
                if pq.shape[0] < T // 2:
                    pq = jnp.concatenate([pq, jnp.zeros((T // 2 - pq.shape[0], T), U32)], axis=0)
                res = _nn(m, pltpu.bitcast(pq, BF))
                num_s[s, i, f0:f0 + rows, :] = res[:rows]
                den.append(res[rows:rows + rows // DH])
            rden_s[t] = gcolv / (jnp.concatenate(den, axis=0) + 1e-6)

        early = EARLY[s]
        for i in range(early):
            read_out(i)
        if s + 1 < NSEG:
            for r, f0 in enumerate(starts):
                rows = mem[r].shape[0]
                vv = jnp.concatenate([v_s[NQ * s + i, f0:f0 + rows, :] for i in range(NQ)], axis=1)
                pk = pk_window(s, f0)
                mem[r] = mem[r] + _nn(vv, pk)
                zsum[r] = zsum[r] + jnp.sum(pk.astype(F32).reshape(L // 8, 8, T), axis=0)
        for i in range(early, NQ):
            read_out(i)

    _wait(cp_wo())
    _start([cp_ya(g) for g in range(NG)])

    tiles = [(i, h, j) for grp in Q_GROUPS for m in range(H // 2) for i in grp
             for h in (2 * m, 2 * m + 1) for j in range(i + 1)]

    def segment(s, carry):
        zeros = [zero_s[9 + i] for i in range(2)]
        sub8 = lax.broadcasted_iota(I32, (8, T), 0)
        lane8 = lax.broadcasted_iota(I32, (8, T), 1)
        t0 = pl.multiple_of(s * L, L)
        qws, mx, pvals, acc, fin, held, ksp = {}, {}, {}, {}, {}, {}, {}

        def q_blocks(i, h):
            f0 = DH * h
            for b in (f0 // 16, f0 // 16 + 1):
                blk = q_s.bitcast(U32)[NQ * s + i, 8 * b:8 * b + 8, :]
                lo, hi = f0 // 2 - 8 * b, (f0 + DH) // 2 - 8 * b
                if lo > 0:
                    blk = jnp.where(sub8 >= lo, blk, jnp.uint32(0))
                if hi < 8:
                    blk = jnp.where(sub8 < hi, blk, jnp.uint32(0))
                yield b, blk

        def q_weights(i, h):
            blocks = [jnp.zeros((8, T), U32)] * 8
            for b, blk in q_blocks(i, h):
                blocks[b % 8] = blk
            return pltpu.bitcast(jnp.concatenate(blocks, axis=0), BF)

        def q_shared(i, m):
            f0 = 2 * DH * m
            blocks = [jnp.zeros((8, T), U32)] * 8
            for b in range(f0 // 16, (f0 + 2 * DH - 1) // 16 + 1):
                blk = q_s.bitcast(U32)[NQ * s + i, 8 * b:8 * b + 8, :]
                row = sub8 + 8 * b - f0 // 2
                in_a = (row >= 0) & (row < DH // 2) & (lane8 < 64)
                in_b = (row >= DH // 2) & (row < DH) & (lane8 >= 64)
                blocks[b % 8] = jnp.where(in_a, pltpu.roll(blk, 64, 1),
                                          jnp.where(in_b, blk, jnp.uint32(0)))
            return pltpu.bitcast(jnp.concatenate(blocks, axis=0), BF)

        def q_split(i, h):
            blocks = [jnp.zeros((8, T), U32)] * 8
            for b, blk in q_blocks(i, h):
                blocks[b % 8] = jnp.where(lane8 >= 32, blk, jnp.uint32(0))
                blocks[(b + 4) % 8] = jnp.where(lane8 < 32, pltpu.roll(blk, 32, 1), jnp.uint32(0))
            return pltpu.bitcast(jnp.concatenate(blocks, axis=0), BF)

        def k_split(win, i, m):
            ku = k_s.bitcast(U32)
            r0 = pl.multiple_of((t0 + T * i) // 2, 8)
            first = ku[win, pl.ds(r0 + 16, 16), :]
            second = pltpu.roll(ku[win, pl.ds(r0 + 48, 16), :], 64, 1)
            lane = lax.broadcasted_iota(I32, (16, T), 1)
            return pltpu.bitcast(jnp.where(((lane - 2 * DH * m) & (T - 1)) < 64, first, second), BF)

        def keep(n, r0, sc):
            i, h, _ = tiles[n]
            m8 = jnp.max(sc.reshape(sc.shape[0] // 8, 8, T), axis=0)
            mx[i, h] = m8 if (i, h) not in mx else jnp.maximum(mx[i, h], m8)
            s_ring[n % RING][0, r0:r0 + sc.shape[0], :] = sc

        def logits(n):
            i, h, j = tiles[n]
            f0 = 2 * DH * (h // 2)
            wb, wa = f0 // T, (f0 + 2 * DH - 1) // T
            win = (wb if wa == wb else NG + wa,)
            if (i, h) not in qws:
                qws[i, h] = q_weights(i, h)
            if j < i:
                keep(n, 0, _nn(_ld(k_s, win, t0 + T * j, T), qws[i, h]))
                return
            keep(n, 0, _nn(_ld(k_s, win, t0 + T * j, 32), qws[i, h]) + mask_s[0:32, :])
            if h % 2 == 0:
                ksp[i] = k_split(win[0], i, h // 2)
            sp = _nn(ksp[i], q_split(i, h))
            keep(n, 32, sp + mask_s[32:64, :])
            keep(n, 96, pltpu.roll(sp, 96, 1) + mask_s[96:T, :])
            if h % 2 == 0:
                sh = _nn(_ld(k_s, win, t0 + T * j + 64, 32), q_shared(i, h // 2))
                keep(n, 64, pltpu.roll(sh, 64, 1) + mask_s[64:96, :])
                keep(n + i + 1, 64, sh + mask_s[64:96, :])

        def probs(n):
            i, h, j = tiles[n]
            if (i, h) not in fin:
                fin[i, h] = jnp.max(mx.pop((i, h)), axis=0, keepdims=True)
            pvals[n] = jnp.exp2(s_ring[n % RING][zeros[0]] - fin[i, h]).astype(BF)

        def values(n):
            i, h, j = tiles[n]
            base = (h // 2) * 2 * DH + (h % 2) * 16
            vv = v_s[NQ * s + j, base:base + 24, :]
            if h % 2 == 0:
                vv = jnp.concatenate([vv[:16], jnp.where(sub8 < 4, vv[16:], 1.0)], axis=0)
            else:
                vv = jnp.concatenate([jnp.where(sub8 >= 4, vv[:8], 1.0), vv[8:]], axis=0)
            o = _nn(vv, pvals.pop(n))
            acc[i, h] = o if j == 0 else acc[i, h] + o
            if j == i:
                a = acc.pop((i, h))
                den = a[DH:DH + 1] if h % 2 == 0 else a[0:1]
                w_dot = (1.0 - g_s[h:h + 1, :]) / den
                w_mem = rden_s[NQ * s + i, h:h + 1, :]
                o = a * w_dot + num_s[s, i, base:base + 24, :] * w_mem
                if h % 2 == 0:
                    ot_s[i][0, base:base + 16, :] = o[:16]
                    held[i] = o[16:]
                else:
                    mid = jnp.where(sub8 < 4, held.pop(i), o[:8])
                    ot_s[i][0, base:base + 24, :] = jnp.concatenate([mid, o[8:]], axis=0)

        def out_proj(i):
            ot = jnp.concatenate([ot_s[i][zeros[1], T * w:T * (w + 1), :].T for w in range(NG)],
                                 axis=1)
            wo = jnp.concatenate([_ld(wo_v, (c,), 0, D) for c in range(NG)], axis=1)
            yb_s[s, T * i:T * (i + 1), :] = _nn(ot.astype(BF), wo).astype(BF)

        n = len(tiles)
        todo = list(OUT_ORDER)
        for tt in range(0, n + LAG_EXP + LAG_PV, STEP):
            for fn, lag in ((logits, 0), (probs, LAG_EXP), (values, LAG_EXP + LAG_PV)):
                for k in range(tt - lag, tt - lag + STEP):
                    if 0 <= k < n:
                        fn(k)
            if len(todo) == NQ and tt + STEP >= n:
                out_proj(todo.pop(0))
        for i in todo:
            if i == NQ - 1:
                cp_yb(s, 0).start()
            out_proj(i)
        cp_yb(s, 1).start()
        return carry

    lax.fori_loop(0, NSEG, segment, 0)

    _wait(cp_conv(NG + 1) + [cp_ya(g) for g in range(NG)])
    _wait([cp_yb(s, part) for s in range(NSEG) for part in range(2)])


@jax.jit
def pallas_concat_heads__ssm_conv_h3__memory_aug_infini_attn__prompt_kernel(
    A_q, A_k, A_v, A_shift_k, A_ssm_k, A_ssm_D, B_x, B_wq, B_wk, B_wv, B_wo, B_beta,
):
    scratch = _scratch()

    def body(*refs):
        _kernel(*refs[:14], **dict(zip(scratch, refs[14:])))

    hbm = pl.BlockSpec(memory_space=pl.ANY)
    out = pl.pallas_call(
        body,
        out_shape=jax.ShapeDtypeStruct((S, 2 * D), BF),
        in_specs=[hbm] * 13,
        out_specs=hbm,
        scratch_shapes=list(scratch.values()),
        compiler_params=pltpu.CompilerParams(vmem_limit_bytes=100 * 1024 * 1024),
        name="h3_infini",
    )(A_q.reshape(S, D), A_k.reshape(S, D), A_v.reshape(S, D), A_shift_k.T, A_ssm_k, A_ssm_D,
      B_x.reshape(S, D), B_wq, B_wk, B_wv, B_wo, B_beta, _DFT)
    return out.reshape(1, S, 2 * D)
```
